```python
import jax
import jax.numpy as jnp

def _softmax(x, axis=-1):
    return jax.nn.softmax(x, axis=axis)

def _gelu(x):
    return jax.nn.gelu(x, approximate=True)

def _silu(x):
    return jax.nn.silu(x)

def _sigmoid(x):
    return jax.nn.sigmoid(x)

def _layernorm(x, axis=-1, eps=1e-05):
    m = jnp.mean(x, axis=axis, keepdims=True)
    v = jnp.var(x, axis=axis, keepdims=True)
    return (x - m) / jnp.sqrt(v + eps)

def _scatter_add(tgt, idx, src, axis=0):
    return tgt.at[idx].add(src)

def _segment_sum(src, seg, n):
    return jax.ops.segment_sum(src, seg, n)

class _Rng:

    def __init__(self, key):
        self._k = key

    def _next(self):
        self._k, sub = jax.random.split(self._k)
        return sub

    def normal(self, shape):
        return jax.random.normal(self._next(), shape, dtype=jnp.bfloat16)

    def randint(self, lo, hi, shape):
        return jax.random.randint(self._next(), shape, lo, hi, dtype=jnp.int32)

    def uniform(self, shape, lo=0.0, hi=1.0):
        return jax.random.uniform(self._next(), shape, jnp.bfloat16, lo, hi)

    def permutation(self, n):
        return jax.random.permutation(self._next(), n)
kernel_name = 'gated_mix__memory_aug_recurrent_mem_tr__sliding_local_dilated__prompt'

def setup_inputs():
    _rng = _Rng(jax.random.key(int.from_bytes(__import__("os").urandom(4), "little")))
    _w = lambda a: (lambda t: t.astype(jnp.bfloat16) if jnp.issubdtype(t.dtype, jnp.floating) else t)(jnp.asarray(a))

    def _A_setup():
        B, S, Dm = (1, 2048, 640)
        H, Dh = (32, 192)
        M, seg = (8, 32)
        seg = min(seg, S)
        S = S // seg * seg
        return {'x': _w((lambda *s: _rng.normal(s) * 0.05)(B, S, Dm)), 'mem0': _w((lambda *s: _rng.normal(s) * 0.05)(B, M, Dm)), 'Wq': _w((lambda *s: _rng.normal(s) * 0.05)(Dm, H, Dh) * Dm ** (-0.5)), 'Wk': _w((lambda *s: _rng.normal(s) * 0.05)(Dm, H, Dh) * Dm ** (-0.5)), 'Wv': _w((lambda *s: _rng.normal(s) * 0.05)(Dm, H, Dh) * Dm ** (-0.5)), 'Wo': _w((lambda *s: _rng.normal(s) * 0.05)(H, Dh, Dm) * (H * Dh) ** (-0.5)), 'seg_len': seg}
    _A_in = _A_setup()

    def _B_setup():
        B, S, D = (1, 2048, 640)
        return {'x': _w((lambda *s: _rng.normal(s) * 0.05)(B, S, D)), 'wqkv': _w((lambda *s: _rng.normal(s) * 0.05)(D, 3 * D)), 'wo': _w((lambda *s: _rng.normal(s) * 0.05)(D, D))}
    _B_in = _B_setup()
    return {'A_x': _A_in['x'], 'A_mem0': _A_in['mem0'], 'A_Wq': _A_in['Wq'], 'A_Wk': _A_in['Wk'], 'A_Wv': _A_in['Wv'], 'A_Wo': _A_in['Wo'], 'A_seg_len': _A_in['seg_len'], 'B_x': _B_in['x'], 'B_wqkv': _B_in['wqkv'], 'B_wo': _B_in['wo'], 'gate_w': _w((lambda *s: _rng.normal(s) * 0.05)(640))}

def reference(A_x, A_mem0, A_Wq, A_Wk, A_Wv, A_Wo, A_seg_len, B_x, B_wqkv, B_wo, gate_w):

    def _A_ref(x, mem0, Wq, Wk, Wv, Wo, seg_len):
        B, S, Dm = x.shape
        H, Dh = (Wq.shape[1], Wq.shape[2])
        M = mem0.shape[1]
        scale = Dh ** (-0.5)
        n_seg = S // seg_len
        L = M + seg_len
        idx = jnp.arange(L)
        mask = (idx[:, None] < M) | (idx[:, None] >= idx[None, :])
        mem = mem0
        outs = []
        for s in range(n_seg):
            xs = x[:, s * seg_len:(s + 1) * seg_len, :].copy()
            h = jnp.concatenate([mem, xs], axis=1)
            q = jnp.einsum('btd,dhe->bhte', h, Wq)
            k = jnp.einsum('btd,dhe->bhte', h, Wk)
            v = jnp.einsum('btd,dhe->bhte', h, Wv)
            scores = jnp.einsum('bhqe,bhke->bhqk', q, k) * scale
            scores = jnp.where(mask[None, None], scores, -1000000000.0)
            p = _softmax(scores, axis=-1)
            o = jnp.einsum('bhqk,bhke->bhqe', p, v)
            o = jnp.einsum('bhte,hed->btd', o, Wo)
            mem = o[:, :M, :].copy()
            outs.append(o[:, M:, :])
        return jnp.concatenate(outs, axis=1)

    def _B_ref(x, wqkv, wo):
        B, S, D = x.shape
        H = 32
        Dh = D // H
        W, dil = (8, 2)
        qkv = (lambda x, *d: x.transpose(*d))((x @ wqkv).reshape(B, S, 3, H, Dh), 2, 0, 3, 1, 4)
        q, k, v = (qkv[0], qkv[1], qkv[2])
        scale = Dh ** (-0.5)
        pos = jnp.arange(S)
        off = jnp.arange(W) * dil
        idx = pos[:, None] - off[None, :]
        mask = idx >= 0
        idx_c = jnp.where(mask, idx, 0).reshape(-1)
        kg = k[:, :, idx_c, :].reshape(B, H, S, W, Dh)
        vg = v[:, :, idx_c, :].reshape(B, H, S, W, Dh)
        logits = jnp.einsum('bhsd,bhswd->bhsw', q, kg) * scale
        logits = jnp.where(mask[None, None, :, :], logits, -1000000000.0)
        attn = _softmax(logits, axis=-1)
        o = jnp.einsum('bhsw,bhswd->bhsd', attn, vg)
        return (lambda x, *d: x.transpose(*d))(o, 0, 2, 1, 3).reshape(B, S, D) @ wo
    x = A_x
    g = _sigmoid((x * gate_w).sum(-1, keepdims=True))
    a = _A_ref(x, A_mem0, A_Wq, A_Wk, A_Wv, A_Wo, A_seg_len)
    b = _B_ref(x, B_wqkv, B_wo)
    return g * a + (1 - g) * b
```

```python
import functools

import jax
import jax.numpy as jnp
import jax.experimental.pallas as pl
import jax.experimental.pallas.tpu as pltpu

_LANES = 128
_B_HEADS = 32
_B_WIN = 8
_B_DIL = 2
_HALO = 16
_MASKED = -1000000000.0
_F32 = jnp.float32
_BF16 = jnp.bfloat16


def _mm(a, b):
    return jax.lax.dot_general(a, b, (((1,), (0,)), ((), ())),
                               preferred_element_type=_F32)


def _mm_nt(a, b):
    return jax.lax.dot_general(a, b, (((1,), (1,)), ((), ())),
                               preferred_element_type=_F32)


def _iota(shape, dim):
    return jax.lax.broadcasted_iota(jnp.int32, shape, dim)


def _kernel(x_hbm, mem0_ref, wq_hbm, wk_hbm, wv_hbm, wo_hbm, bqkv_hbm, bwo_hbm,
            gate_ref, out_hbm,
            x_ref, stage_ref, wt_ref, wo_ref, bqkv_ref, bwo_ref, bqkvp_ref,
            bwo32_ref, bwop_ref, q_ref, k_ref, v_ref, att_ref, b_ref, o_ref,
            out_ref, in_sem, w_sem, wo_sem, out_sem,
            *, seg, dh, t_chunk, t_sub, out_group):
    S, D = x_ref.shape
    M = mem0_ref.shape[0]
    L = M + seg
    n_seg = S // seg
    n_pair, pw = wt_ref.shape[0], 2 * dh
    n_chunk = S // t_chunk
    ppc = n_pair // n_chunk
    n_tile = D // _LANES
    bdh = D // _B_HEADS

    cp_bqkv = pltpu.make_async_copy(bqkv_hbm, bqkv_ref, in_sem.at[0])
    cp_x = pltpu.make_async_copy(x_hbm, x_ref, in_sem.at[1])
    cp_bwo = pltpu.make_async_copy(bwo_hbm, bwo_ref, in_sem.at[2])

    def cp_w(c, m):
        src = (wq_hbm, wk_hbm, wv_hbm)[m]
        rows = pl.ds(c * ppc * pw, ppc * pw)
        return pltpu.make_async_copy(src.at[rows], stage_ref.at[m, rows],
                                     w_sem.at[c, m])

    cp_wo = pltpu.make_async_copy(wo_hbm, wo_ref, wo_sem.at[0])

    cp_bqkv.start()
    cp_x.start()
    cp_bwo.start()
    for c in range(n_chunk):
        for m in range(3):
            cp_w(c, m).start()
    cp_wo.start()

    src = _iota((D, D), 0)
    dst = _iota((D, D), 1)
    perm = (src == (dst % _B_HEADS) * bdh + dst // _B_HEADS)
    perm = jnp.where(perm, 1.0, 0.0).astype(_BF16)
    cp_bqkv.wait()
    for j in range(3):
        cols = slice(j * D, (j + 1) * D)
        bqkvp_ref[:, cols] = _mm(bqkv_ref[:, cols], perm).astype(_BF16)
    cp_bwo.wait()
    for j in range(n_tile):
        cols = slice(j * _LANES, (j + 1) * _LANES)
        bwo32_ref[j] = bwo_ref[:, cols].astype(_F32)
        for d in range(bdh):
            bwop_ref[d * _B_HEADS:(d + 1) * _B_HEADS, cols] = bwo32_ref[
                j, pl.ds(d, _B_HEADS, stride=bdh), :].astype(_BF16)
    cp_x.wait()

    b_scale = float(bdh) ** -0.5

    def b_chunk(c, carry):
        t0 = pl.multiple_of(c * t_chunk, t_chunk)
        xc = x_ref[pl.ds(t0, t_chunk), :]
        q_ref[...] = _mm(xc, bqkvp_ref[:, 0:D]) * b_scale
        k_ref[_HALO:, :] = _mm(xc, bqkvp_ref[:, D:2 * D])
        v_ref[_HALO:, :] = _mm(xc, bqkvp_ref[:, 2 * D:3 * D])

        @pl.when(c == 0)
        def _():
            k_ref[0:_HALO, :] = jnp.broadcast_to(k_ref[_HALO:_HALO + 1, :], (_HALO, D))
            v_ref[0:_HALO, :] = jnp.broadcast_to(v_ref[_HALO:_HALO + 1, :], (_HALO, D))

        for r in range(0, t_chunk, t_sub):
            q = q_ref[r:r + t_sub, :]
            logits = []
            for w in range(_B_WIN):
                a = _HALO + r - w * _B_DIL
                prod = q * k_ref[a:a + t_sub, :]
                s = prod[:, 0:_LANES]
                for j in range(1, n_tile):
                    s = s + prod[:, j * _LANES:(j + 1) * _LANES]
                s = s + pltpu.roll(s, 2 * _B_HEADS, 1)
                s = s + pltpu.roll(s, _B_HEADS, 1)
                if r < w * _B_DIL:
                    pos = t0 + r + _iota((t_sub, _LANES), 0)
                    s = jnp.where(pos >= w * _B_DIL, s, _MASKED)
                logits.append(s)
            mx = functools.reduce(jnp.maximum, logits)
            es = [jnp.exp(s - mx) for s in logits]
            inv = 1.0 / functools.reduce(jnp.add, es)
            ps = [e * inv for e in es]
            for j in range(n_tile):
                cols = slice(j * _LANES, (j + 1) * _LANES)
                acc = None
                for w in range(_B_WIN):
                    a = _HALO + r - w * _B_DIL
                    t = ps[w] * v_ref[a:a + t_sub, cols]
                    acc = t if acc is None else acc + t
                att_ref[r:r + t_sub, cols] = acc
        b_ref[pl.ds(t0, t_chunk), :] = _mm(att_ref[...], bwop_ref[...])
        k_ref[0:_HALO, :] = k_ref[t_chunk:, :]
        v_ref[0:_HALO, :] = v_ref[t_chunk:, :]

        for m in range(3):
            cp_w(c, m).wait()
        for i in range(ppc):
            p = c * ppc + i
            rows = pl.ds(pl.multiple_of(p * pw, pw), pw)
            for m in range(3):
                wt_ref[p, :, m * pw:(m + 1) * pw] = stage_ref[m, rows, :].T
        return carry

    jax.lax.fori_loop(0, n_chunk, b_chunk, 0)
    cp_wo.wait()

    a_scale = float(dh) ** -0.5
    out_rows = out_group * seg

    def cp_out(g):
        rows = pl.ds(pl.multiple_of(g * out_rows, out_rows), out_rows)
        return pltpu.make_async_copy(out_ref.at[rows], out_hbm.at[rows],
                                     out_sem.at[0])

    def block_diag(t):
        first = _iota((L, pw), 1) < dh
        return jnp.concatenate(
            [jnp.where(first, t, 0.0), jnp.where(first, 0.0, t)], axis=0
        ).astype(_BF16)

    def a_step(s, mem):
        r0 = pl.multiple_of(s * seg, seg)
        xs = x_ref[pl.ds(r0, seg), :].astype(_F32)
        h = jnp.concatenate([mem, xs], axis=0)

        row = _iota((L, 2 * L), 0)
        col = _iota((L, 2 * L), 1)
        first = col < L
        key = jnp.where(first, col, col - L)
        visible = (row < M) | (row >= key)

        def project(p):
            qkv = _mm(h, wt_ref[p])
            return qkv[:, 0:pw], block_diag(qkv[:, pw:2 * pw]), block_diag(qkv[:, 2 * pw:])

        def softmax(q, kbd):
            sc = jnp.where(visible, _mm_nt(q, kbd) * a_scale, _MASKED)
            m0 = jnp.max(jnp.where(first, sc, -jnp.inf), axis=1, keepdims=True)
            m1 = jnp.max(jnp.where(first, -jnp.inf, sc), axis=1, keepdims=True)
            e = jnp.exp(sc - jnp.where(first, m0, m1))
            s0 = jnp.sum(jnp.where(first, e, 0.0), axis=1, keepdims=True)
            s1 = jnp.sum(jnp.where(first, 0.0, e), axis=1, keepdims=True)
            return e / jnp.where(first, s0, s1)

        proj, prob = {}, {}
        for p in range(n_pair + 2):
            if p < n_pair:
                proj[p] = project(p)
            if 0 <= p - 1 < n_pair:
                prob[p - 1] = softmax(proj[p - 1][0], proj[p - 1][1])
            if 0 <= p - 2 < n_pair:
                o_ref[:, (p - 2) * pw:(p - 1) * pw] = _mm(prob[p - 2], proj[p - 2][2])
        res = _mm(o_ref[...], wo_ref[...])

        g = jax.nn.sigmoid(jnp.sum(xs * gate_ref[...].astype(_F32), axis=1, keepdims=True))
        out_ref[pl.ds(r0, seg), :] = (
            g * res[M:, :] + (1.0 - g) * b_ref[pl.ds(r0, seg), :]).astype(out_ref.dtype)

        @pl.when(s % out_group == out_group - 1)
        def _():
            cp_out(s // out_group).start()

        return res[0:M, :]

    jax.lax.fori_loop(0, n_seg, a_step, mem0_ref[...].astype(_F32))
    pltpu.make_async_copy(out_ref, out_hbm, out_sem.at[0]).wait()


@functools.partial(jax.jit, static_argnames=("A_seg_len",))
def pallas_gated_mix__memory_aug_recurrent_mem_tr__sliding_local_dilated__prompt_kernel(
    A_x: jax.Array,
    A_mem0: jax.Array,
    A_Wq: jax.Array,
    A_Wk: jax.Array,
    A_Wv: jax.Array,
    A_Wo: jax.Array,
    A_seg_len: int,
    B_x: jax.Array,
    B_wqkv: jax.Array,
    B_wo: jax.Array,
    gate_w: jax.Array,
):
    del B_x
    _, S, D = A_x.shape
    _, H, dh = A_Wq.shape
    M = A_mem0.shape[1]
    seg = int(A_seg_len)
    L = M + seg
    E = H * dh
    n_pair = H // 2
    t_chunk, t_sub, out_group = 256, 32, 8
    n_chunk = S // t_chunk

    def rows_major(w):
        return jnp.transpose(w, (1, 2, 0)).reshape(E, D)

    hbm = pl.BlockSpec(memory_space=pl.ANY)
    vmem = pl.BlockSpec(memory_space=pltpu.VMEM)
    out = pl.pallas_call(
        functools.partial(_kernel, seg=seg, dh=dh, t_chunk=t_chunk, t_sub=t_sub,
                          out_group=out_group),
        out_shape=jax.ShapeDtypeStruct((S, D), A_x.dtype),
        in_specs=[hbm, vmem, hbm, hbm, hbm, hbm, hbm, hbm, vmem],
        out_specs=hbm,
        scratch_shapes=[
            pltpu.VMEM((S, D), _BF16),
            pltpu.VMEM((3, E, D), _BF16),
            pltpu.VMEM((n_pair, D, 6 * dh), _BF16),
            pltpu.VMEM((E, D), _BF16),
            pltpu.VMEM((D, 3 * D), _BF16),
            pltpu.VMEM((D, D), _BF16),
            pltpu.VMEM((D, 3 * D), _BF16),
            pltpu.VMEM((D // _LANES, D, _LANES), _F32),
            pltpu.VMEM((D, D), _BF16),
            pltpu.VMEM((t_chunk, D), _F32),
            pltpu.VMEM((_HALO + t_chunk, D), _F32),
            pltpu.VMEM((_HALO + t_chunk, D), _F32),
            pltpu.VMEM((t_chunk, D), _F32),
            pltpu.VMEM((S, D), _F32),
            pltpu.VMEM((L, E), _F32),
            pltpu.VMEM((S, D), A_x.dtype),
            pltpu.SemaphoreType.DMA((3,)),
            pltpu.SemaphoreType.DMA((n_chunk, 3)),
            pltpu.SemaphoreType.DMA((1,)),
            pltpu.SemaphoreType.DMA((1,)),
        ],
        compiler_params=pltpu.CompilerParams(vmem_limit_bytes=110 * 1024 * 1024),
    )(A_x.reshape(S, D), A_mem0.reshape(M, D), rows_major(A_Wq), rows_major(A_Wk),
      rows_major(A_Wv), A_Wo.reshape(E, D), B_wqkv, B_wo, gate_w.reshape(1, D))
    return out.reshape(1, S, D)
```

```python
import functools

import jax
import jax.numpy as jnp
import jax.experimental.pallas as pl
import jax.experimental.pallas.tpu as pltpu

_LANES = 128
_B_HEADS = 32
_B_WIN = 8
_B_DIL = 2
_HALO = 16
_MASKED = -1000000000.0
_F32 = jnp.float32
_BF16 = jnp.bfloat16


def _mm(a, b):
    return jax.lax.dot_general(a, b, (((1,), (0,)), ((), ())),
                               preferred_element_type=_F32)


def _mm_nt(a, b):
    return jax.lax.dot_general(a, b, (((1,), (1,)), ((), ())),
                               preferred_element_type=_F32)


def _iota(shape, dim):
    return jax.lax.broadcasted_iota(jnp.int32, shape, dim)


def _kernel(x_hbm, mem0_ref, wq_hbm, wk_hbm, wv_hbm, wo_hbm, bqkv_hbm, bwo_hbm,
            gate_ref, out_hbm,
            x_ref, stage_ref, wt_ref, wo_ref, bqkv_ref, bwo_ref, bqkvp_ref,
            bwo32_ref, bwop_ref, q_ref, k_ref, v_ref, att_ref, b_ref, o_ref,
            out_ref, in_sem, w_sem, wo_sem, out_sem,
            *, seg, dh, t_chunk, t_sub, out_group, ahead):
    S, D = x_ref.shape
    M = mem0_ref.shape[0]
    L = M + seg
    n_seg = S // seg
    n_pair, pw = wt_ref.shape[0], 2 * dh
    n_chunk = S // t_chunk
    ppc = n_pair // n_chunk
    n_tile = D // _LANES
    bdh = D // _B_HEADS

    cp_bqkv = pltpu.make_async_copy(bqkv_hbm, bqkv_ref, in_sem.at[0])
    cp_x = pltpu.make_async_copy(x_hbm, x_ref, in_sem.at[1])
    cp_bwo = pltpu.make_async_copy(bwo_hbm, bwo_ref, in_sem.at[2])

    def cp_w(c, m):
        src = (wq_hbm, wk_hbm, wv_hbm)[m]
        rows = pl.ds(c * ppc * pw, ppc * pw)
        return pltpu.make_async_copy(src.at[rows], stage_ref.at[m, rows],
                                     w_sem.at[c, m])

    cp_wo = pltpu.make_async_copy(wo_hbm, wo_ref, wo_sem.at[0])

    def start_w(c):
        if c < n_chunk:
            for m in range(3):
                cp_w(c, m).start()
        elif c == n_chunk:
            cp_wo.start()

    cp_bqkv.start()
    cp_x.start()
    cp_bwo.start()

    src = _iota((D, D), 0)
    dst = _iota((D, D), 1)
    perm = (src == (dst % _B_HEADS) * bdh + dst // _B_HEADS)
    perm = jnp.where(perm, 1.0, 0.0).astype(_BF16)
    cp_bqkv.wait()
    for c in range(ahead):
        start_w(c)
    for j in range(3):
        cols = slice(j * D, (j + 1) * D)
        bqkvp_ref[:, cols] = _mm(bqkv_ref[:, cols], perm).astype(_BF16)
    cp_bwo.wait()
    for j in range(n_tile):
        cols = slice(j * _LANES, (j + 1) * _LANES)
        bwo32_ref[j] = bwo_ref[:, cols].astype(_F32)
        for d in range(bdh):
            bwop_ref[d * _B_HEADS:(d + 1) * _B_HEADS, cols] = bwo32_ref[
                j, pl.ds(d, _B_HEADS, stride=bdh), :].astype(_BF16)
    cp_x.wait()

    b_scale = float(bdh) ** -0.5

    def b_project(c):
        xc = x_ref[c * t_chunk:(c + 1) * t_chunk, :]
        q = _mm(xc, bqkvp_ref[:, 0:D]) * b_scale
        k = _mm(xc, bqkvp_ref[:, D:2 * D])
        v = _mm(xc, bqkvp_ref[:, 2 * D:3 * D])
        rows = slice(_HALO + c * t_chunk, _HALO + (c + 1) * t_chunk)
        for j in range(n_tile):
            cols = slice(j * _LANES, (j + 1) * _LANES)
            q_ref[j, c * t_chunk:(c + 1) * t_chunk, :] = q[:, cols]
            k_ref[j, rows, :] = k[:, cols]
            v_ref[j, rows, :] = v[:, cols]
            if c == 0:
                k_ref[j, 0:_HALO, :] = jnp.broadcast_to(k[0:1, cols], (_HALO, _LANES))
                v_ref[j, 0:_HALO, :] = jnp.broadcast_to(v[0:1, cols], (_HALO, _LANES))

    def b_attend(c):
        for r in range(c * t_chunk, (c + 1) * t_chunk, t_sub):
            q = [q_ref[j, r:r + t_sub, :] for j in range(n_tile)]
            logits = []
            for w in range(_B_WIN):
                a = _HALO + r - w * _B_DIL
                s = functools.reduce(jnp.add, [
                    q[j] * k_ref[j, pl.ds(a, t_sub), :] for j in range(n_tile)])
                s = s + pltpu.roll(s, 2 * _B_HEADS, 1)
                s = s + pltpu.roll(s, _B_HEADS, 1)
                if r < w * _B_DIL:
                    pos = r + _iota((t_sub, _LANES), 0)
                    s = jnp.where(pos >= w * _B_DIL, s, _MASKED)
                logits.append(s)
            mx = functools.reduce(jnp.maximum, logits)
            es = [jnp.exp(s - mx) for s in logits]
            inv = 1.0 / functools.reduce(jnp.add, es)
            for j in range(n_tile):
                acc = functools.reduce(jnp.add, [
                    es[w] * v_ref[j, pl.ds(_HALO + r - w * _B_DIL, t_sub), :]
                    for w in range(_B_WIN)])
                att_ref[r:r + t_sub, j * _LANES:(j + 1) * _LANES] = (acc * inv).astype(_BF16)

    def b_output(c):
        rows = slice(c * t_chunk, (c + 1) * t_chunk)
        b_ref[rows, :] = _mm(att_ref[rows, :], bwop_ref[...])

    def transpose_w(c):
        for m in range(3):
            cp_w(c, m).wait()
        start_w(c + ahead)
        for p in range(c * ppc, (c + 1) * ppc):
            for m in range(3):
                wt_ref[p, :, m * pw:(m + 1) * pw] = stage_ref[m, p * pw:(p + 1) * pw, :].T

    for i in range(n_chunk + 2):
        if 1 <= i <= n_chunk:
            transpose_w(i - 1)
        if i < n_chunk:
            b_project(i)
        if 1 <= i <= n_chunk:
            b_attend(i - 1)
        if i >= 2:
            b_output(i - 2)
    cp_wo.wait()

    a_scale = float(dh) ** -0.5
    out_rows = out_group * seg

    def cp_out(g):
        rows = pl.ds(pl.multiple_of(g * out_rows, out_rows), out_rows)
        return pltpu.make_async_copy(out_ref.at[rows], out_hbm.at[rows],
                                     out_sem.at[0])

    def block_diag(t):
        first = _iota((L, pw), 1) < dh
        return jnp.concatenate(
            [jnp.where(first, t, 0.0), jnp.where(first, 0.0, t)], axis=0
        ).astype(_BF16)

    def a_step(s, mem):
        r0 = pl.multiple_of(s * seg, seg)
        xs = x_ref[pl.ds(r0, seg), :].astype(_F32)
        h = jnp.concatenate([mem, xs], axis=0)

        row = _iota((L, 2 * L), 0)
        col = _iota((L, 2 * L), 1)
        first = col < L
        key = jnp.where(first, col, col - L)
        visible = (row < M) | (row >= key)

        def project(p):
            qkv = _mm(h, wt_ref[p])
            return qkv[:, 0:pw], block_diag(qkv[:, pw:2 * pw]), block_diag(qkv[:, 2 * pw:])

        def softmax(q, kbd):
            sc = jnp.where(visible, _mm_nt(q, kbd) * a_scale, _MASKED)
            m0 = jnp.max(jnp.where(first, sc, -jnp.inf), axis=1, keepdims=True)
            m1 = jnp.max(jnp.where(first, -jnp.inf, sc), axis=1, keepdims=True)
            e = jnp.exp(sc - jnp.where(first, m0, m1))
            s0 = jnp.sum(jnp.where(first, e, 0.0), axis=1, keepdims=True)
            s1 = jnp.sum(jnp.where(first, 0.0, e), axis=1, keepdims=True)
            return e / jnp.where(first, s0, s1)

        proj, prob = {}, {}
        for p in range(n_pair + 2):
            if p < n_pair:
                proj[p] = project(p)
            if 0 <= p - 1 < n_pair:
                prob[p - 1] = softmax(proj[p - 1][0], proj[p - 1][1])
            if 0 <= p - 2 < n_pair:
                o_ref[:, (p - 2) * pw:(p - 1) * pw] = _mm(prob[p - 2], proj[p - 2][2])
        res = _mm(o_ref[...], wo_ref[...])

        g = jax.nn.sigmoid(jnp.sum(xs * gate_ref[...].astype(_F32), axis=1, keepdims=True))
        out_ref[pl.ds(r0, seg), :] = (
            g * res[M:, :] + (1.0 - g) * b_ref[pl.ds(r0, seg), :]).astype(out_ref.dtype)

        @pl.when(s % out_group == out_group - 1)
        def _():
            cp_out(s // out_group).start()

        return res[0:M, :]

    jax.lax.fori_loop(0, n_seg, a_step, mem0_ref[...].astype(_F32))
    pltpu.make_async_copy(out_ref, out_hbm, out_sem.at[0]).wait()


@functools.partial(jax.jit, static_argnames=("A_seg_len",))
def pallas_gated_mix__memory_aug_recurrent_mem_tr__sliding_local_dilated__prompt_kernel(
    A_x: jax.Array,
    A_mem0: jax.Array,
    A_Wq: jax.Array,
    A_Wk: jax.Array,
    A_Wv: jax.Array,
    A_Wo: jax.Array,
    A_seg_len: int,
    B_x: jax.Array,
    B_wqkv: jax.Array,
    B_wo: jax.Array,
    gate_w: jax.Array,
):
    del B_x
    _, S, D = A_x.shape
    _, H, dh = A_Wq.shape
    M = A_mem0.shape[1]
    seg = int(A_seg_len)
    L = M + seg
    E = H * dh
    n_pair = H // 2
    t_chunk, t_sub, out_group, ahead = 256, 32, 8, 2
    n_chunk = S // t_chunk

    def rows_major(w):
        return jnp.transpose(w, (1, 2, 0)).reshape(E, D)

    hbm = pl.BlockSpec(memory_space=pl.ANY)
    vmem = pl.BlockSpec(memory_space=pltpu.VMEM)
    out = pl.pallas_call(
        functools.partial(_kernel, seg=seg, dh=dh, t_chunk=t_chunk, t_sub=t_sub,
                          out_group=out_group, ahead=ahead),
        out_shape=jax.ShapeDtypeStruct((S, D), A_x.dtype),
        in_specs=[hbm, vmem, hbm, hbm, hbm, hbm, hbm, hbm, vmem],
        out_specs=hbm,
        scratch_shapes=[
            pltpu.VMEM((S, D), _BF16),
            pltpu.VMEM((3, E, D), _BF16),
            pltpu.VMEM((n_pair, D, 6 * dh), _BF16),
            pltpu.VMEM((E, D), _BF16),
            pltpu.VMEM((D, 3 * D), _BF16),
            pltpu.VMEM((D, D), _BF16),
            pltpu.VMEM((D, 3 * D), _BF16),
            pltpu.VMEM((D // _LANES, D, _LANES), _F32),
            pltpu.VMEM((D, D), _BF16),
            pltpu.VMEM((D // _LANES, S, _LANES), _F32),
            pltpu.VMEM((D // _LANES, _HALO + S, _LANES), _F32),
            pltpu.VMEM((D // _LANES, _HALO + S, _LANES), _F32),
            pltpu.VMEM((S, D), _BF16),
            pltpu.VMEM((S, D), _F32),
            pltpu.VMEM((L, E), _F32),
            pltpu.VMEM((S, D), A_x.dtype),
            pltpu.SemaphoreType.DMA((3,)),
            pltpu.SemaphoreType.DMA((n_chunk, 3)),
            pltpu.SemaphoreType.DMA((1,)),
            pltpu.SemaphoreType.DMA((1,)),
        ],
        compiler_params=pltpu.CompilerParams(vmem_limit_bytes=110 * 1024 * 1024),
    )(A_x.reshape(S, D), A_mem0.reshape(M, D), rows_major(A_Wq), rows_major(A_Wk),
      rows_major(A_Wv), A_Wo.reshape(E, D), B_wqkv, B_wo, gate_w.reshape(1, D))
    return out.reshape(1, S, D)
```

```python
import functools

import jax
import jax.numpy as jnp
import jax.experimental.pallas as pl
import jax.experimental.pallas.tpu as pltpu

_LANES = 128
_B_HEADS = 32
_B_WIN = 8
_B_DIL = 2
_HALO = 16
_MASKED = -1000000000.0
_F32 = jnp.float32
_BF16 = jnp.bfloat16


def _mm(a, b):
    return jax.lax.dot_general(a, b, (((1,), (0,)), ((), ())),
                               preferred_element_type=_F32)


def _mm_nt(a, b):
    return jax.lax.dot_general(a, b, (((1,), (1,)), ((), ())),
                               preferred_element_type=_F32)


def _iota(shape, dim):
    return jax.lax.broadcasted_iota(jnp.int32, shape, dim)


def _kernel(x_hbm, mem0_ref, wq_hbm, wk_hbm, wv_hbm, wo_hbm, bqkv_hbm, bwo_hbm,
            gate_ref, out_hbm,
            x_ref, stage_ref, wt_ref, wo_ref, bqkv_ref, bwo_ref, b32_ref,
            bp_ref, qkv_ref, att_ref, b_ref, o_ref,
            out_ref, in_sem, w_sem, wo_sem, out_sem,
            *, seg, dh, t_chunk, t_sub, out_group, ahead, x_chunks, w_lag):
    S, D = x_ref.shape
    M = mem0_ref.shape[0]
    L = M + seg
    n_seg = S // seg
    n_pair, pw = wt_ref.shape[0], 2 * dh
    n_chunk = S // t_chunk
    ppc = n_pair // n_chunk
    n_tile = D // _LANES
    bdh = D // _B_HEADS

    x_head = x_chunks * t_chunk
    cp_bqkv = pltpu.make_async_copy(bqkv_hbm, bqkv_ref, in_sem.at[0])
    cp_x0 = pltpu.make_async_copy(x_hbm.at[0:x_head], x_ref.at[0:x_head], in_sem.at[1])
    cp_x1 = pltpu.make_async_copy(x_hbm.at[x_head:S], x_ref.at[x_head:S], in_sem.at[2])
    cp_bwo = pltpu.make_async_copy(bwo_hbm, bwo_ref, in_sem.at[3])

    def cp_w(c, m):
        src = (wq_hbm, wk_hbm, wv_hbm)[m]
        rows = pl.ds(c * ppc * pw, ppc * pw)
        return pltpu.make_async_copy(src.at[rows], stage_ref.at[m, rows],
                                     w_sem.at[c, m])

    cp_wo = pltpu.make_async_copy(wo_hbm, wo_ref, wo_sem.at[0])

    def start_w(c):
        if c < n_chunk:
            for m in range(3):
                cp_w(c, m).start()
        elif c == n_chunk:
            cp_wo.start()

    cp_bqkv.start()
    cp_x0.start()

    def reorder_rows(m, tile):
        for j in range(n_tile):
            b32_ref[m, j] = tile(j).astype(_F32)
            for d in range(bdh):
                bp_ref[m, d * _B_HEADS:(d + 1) * _B_HEADS, j * _LANES:(j + 1) * _LANES] = (
                    b32_ref[m, j, pl.ds(d, _B_HEADS, stride=bdh), :].astype(_BF16))

    cp_bqkv.wait()
    cp_x1.start()
    cp_bwo.start()
    for c in range(ahead - 1):
        start_w(c)
    cp_x0.wait()

    b_scale = float(bdh) ** -0.5

    def b_project(c, m):
        if c == 0:
            reorder_rows(m, lambda j: bqkv_ref[j * _LANES:(j + 1) * _LANES,
                                               m * D:(m + 1) * D].T)
        y = _mm_nt(x_ref[c * t_chunk:(c + 1) * t_chunk, :], bp_ref[m])
        if m == 0:
            y = y * b_scale
        for j in range(n_tile):
            cols = slice(j * _LANES, (j + 1) * _LANES)
            qkv_ref[m, j, _HALO + c * t_chunk:_HALO + (c + 1) * t_chunk, :] = y[:, cols]
            if c == 0 and m > 0:
                qkv_ref[m, j, 0:_HALO, :] = jnp.broadcast_to(y[0:1, cols], (_HALO, _LANES))

    def b_attend(r):
        def rows(m, j, w):
            return qkv_ref[m, j, pl.ds(_HALO + r - w * _B_DIL, t_sub), :]

        q = [rows(0, j, 0) for j in range(n_tile)]
        logits = []
        for w in range(_B_WIN):
            s = functools.reduce(jnp.add, [q[j] * rows(1, j, w) for j in range(n_tile)])
            s = s + pltpu.roll(s, 2 * _B_HEADS, 1)
            s = s + pltpu.roll(s, _B_HEADS, 1)
            if r < w * _B_DIL:
                pos = r + _iota((t_sub, _LANES), 0)
                s = jnp.where(pos >= w * _B_DIL, s, _MASKED)
            logits.append(s)
        mx = functools.reduce(jnp.maximum, logits)
        es = [jnp.exp(s - mx) for s in logits]
        inv = 1.0 / functools.reduce(jnp.add, es)
        for j in range(n_tile):
            acc = functools.reduce(jnp.add, [es[w] * rows(2, j, w) for w in range(_B_WIN)])
            att_ref[r:r + t_sub, j * _LANES:(j + 1) * _LANES] = (acc * inv).astype(_BF16)

    def b_output(c):
        if c == 0:
            reorder_rows(3, lambda j: bwo_ref[:, j * _LANES:(j + 1) * _LANES])
        rows = slice(c * t_chunk, (c + 1) * t_chunk)
        b_ref[rows, :] = _mm(att_ref[rows, :], bp_ref[3])

    def transpose_w(c, m):
        for p in range(c * ppc, (c + 1) * ppc):
            wt_ref[p, :, m * pw:(m + 1) * pw] = stage_ref[m, p * pw:(p + 1) * pw, :].T

    n_sub = t_chunk // t_sub
    subs = [n_sub * f // 8 for f in (0, 4, 8, 8, 8)]
    for i in range(n_chunk + 2):
        c = i - w_lag
        if i == w_lag - 1:
            start_w(ahead - 1)
        if i == min(x_chunks, 2):
            cp_x1.wait()
            cp_bwo.wait()
        if 0 <= c < n_chunk:
            for m in range(3):
                cp_w(c, m).wait()
            start_w(c + ahead)
        for m in range(4):
            if 1 <= i <= n_chunk:
                for u in range(subs[m], subs[m + 1]):
                    b_attend((i - 1) * t_chunk + u * t_sub)
            if m < 3 and 0 <= c < n_chunk:
                transpose_w(c, m)
            if m < 3 and i < n_chunk:
                b_project(i, m)
            if m == 3 and i >= 2:
                b_output(i - 2)

    a_scale = float(dh) ** -0.5
    out_rows = out_group * seg

    def cp_out(g):
        rows = pl.ds(pl.multiple_of(g * out_rows, out_rows), out_rows)
        return pltpu.make_async_copy(out_ref.at[rows], out_hbm.at[rows],
                                     out_sem.at[0])

    def block_diag(t):
        first = _iota((L, pw), 1) < dh
        return jnp.concatenate(
            [jnp.where(first, t, 0.0), jnp.where(first, 0.0, t)], axis=0
        ).astype(_BF16)

    def a_step(s, mem, first_step=False):
        r0 = 0 if first_step else pl.multiple_of(s * seg, seg)
        xs = x_ref[pl.ds(r0, seg), :].astype(_F32)
        h = jnp.concatenate([mem, xs], axis=0)

        row = _iota((L, 2 * L), 0)
        col = _iota((L, 2 * L), 1)
        first = col < L
        key = jnp.where(first, col, col - L)
        visible = (row < M) | (row >= key)

        def project(p):
            qkv = _mm(h, wt_ref[p])
            return qkv[:, 0:pw], block_diag(qkv[:, pw:2 * pw]), block_diag(qkv[:, 2 * pw:])

        def softmax(q, kbd):
            sc = jnp.where(visible, _mm_nt(q, kbd) * a_scale, _MASKED)
            m0 = jnp.max(jnp.where(first, sc, -jnp.inf), axis=1, keepdims=True)
            m1 = jnp.max(jnp.where(first, -jnp.inf, sc), axis=1, keepdims=True)
            e = jnp.exp(sc - jnp.where(first, m0, m1))
            s0 = jnp.sum(jnp.where(first, e, 0.0), axis=1, keepdims=True)
            s1 = jnp.sum(jnp.where(first, 0.0, e), axis=1, keepdims=True)
            return e / jnp.where(first, s0, s1)

        proj, prob = {}, {}
        for p in range(n_pair + 2):
            if p < n_pair:
                proj[p] = project(p)
            if 0 <= p - 1 < n_pair:
                prob[p - 1] = softmax(proj[p - 1][0], proj[p - 1][1])
            if 0 <= p - 2 < n_pair:
                o_ref[:, (p - 2) * pw:(p - 1) * pw] = _mm(prob[p - 2], proj[p - 2][2])
        if first_step:
            cp_wo.wait()
        res = _mm(o_ref[...], wo_ref[...])

        g = jax.nn.sigmoid(jnp.sum(xs * gate_ref[...].astype(_F32), axis=1, keepdims=True))
        out_ref[pl.ds(r0, seg), :] = (
            g * res[M:, :] + (1.0 - g) * b_ref[pl.ds(r0, seg), :]).astype(out_ref.dtype)

        if not first_step:
            @pl.when(s % out_group == out_group - 1)
            def _():
                cp_out(s // out_group).start()

        return res[0:M, :]

    mem = a_step(0, mem0_ref[...].astype(_F32), first_step=True)
    jax.lax.fori_loop(1, n_seg, a_step, mem)
    pltpu.make_async_copy(out_ref, out_hbm, out_sem.at[0]).wait()


@functools.partial(jax.jit, static_argnames=("A_seg_len",))
def pallas_gated_mix__memory_aug_recurrent_mem_tr__sliding_local_dilated__prompt_kernel(
    A_x: jax.Array,
    A_mem0: jax.Array,
    A_Wq: jax.Array,
    A_Wk: jax.Array,
    A_Wv: jax.Array,
    A_Wo: jax.Array,
    A_seg_len: int,
    B_x: jax.Array,
    B_wqkv: jax.Array,
    B_wo: jax.Array,
    gate_w: jax.Array,
):
    del B_x
    _, S, D = A_x.shape
    _, H, dh = A_Wq.shape
    M = A_mem0.shape[1]
    seg = int(A_seg_len)
    L = M + seg
    E = H * dh
    n_pair = H // 2
    t_chunk, t_sub, out_group, ahead, x_chunks, w_lag = 256, 128, 8, 3, 2, 1
    n_chunk = S // t_chunk

    def rows_major(w):
        return jnp.transpose(w, (1, 2, 0)).reshape(E, D)

    hbm = pl.BlockSpec(memory_space=pl.ANY)
    vmem = pl.BlockSpec(memory_space=pltpu.VMEM)
    out = pl.pallas_call(
        functools.partial(_kernel, seg=seg, dh=dh, t_chunk=t_chunk, t_sub=t_sub,
                          out_group=out_group, ahead=ahead, x_chunks=x_chunks,
                          w_lag=w_lag),
        out_shape=jax.ShapeDtypeStruct((S, D), A_x.dtype),
        in_specs=[hbm, vmem, hbm, hbm, hbm, hbm, hbm, hbm, vmem],
        out_specs=hbm,
        scratch_shapes=[
            pltpu.VMEM((S, D), _BF16),
            pltpu.VMEM((3, E, D), _BF16),
            pltpu.VMEM((n_pair, D, 6 * dh), _BF16),
            pltpu.VMEM((E, D), _BF16),
            pltpu.VMEM((D, 3 * D), _BF16),
            pltpu.VMEM((D, D), _BF16),
            pltpu.VMEM((4, D // _LANES, D, _LANES), _F32),
            pltpu.VMEM((4, D, D), _BF16),
            pltpu.VMEM((3, D // _LANES, _HALO + S, _LANES), _F32),
            pltpu.VMEM((S, D), _BF16),
            pltpu.VMEM((S, D), _F32),
            pltpu.VMEM((L, E), _F32),
            pltpu.VMEM((S, D), A_x.dtype),
            pltpu.SemaphoreType.DMA((4,)),
            pltpu.SemaphoreType.DMA((n_chunk, 3)),
            pltpu.SemaphoreType.DMA((1,)),
            pltpu.SemaphoreType.DMA((1,)),
        ],
        compiler_params=pltpu.CompilerParams(vmem_limit_bytes=110 * 1024 * 1024),
    )(A_x.reshape(S, D), A_mem0.reshape(M, D), rows_major(A_Wq), rows_major(A_Wk),
      rows_major(A_Wv), A_Wo.reshape(E, D), B_wqkv, B_wo, gate_w.reshape(1, D))
    return out.reshape(1, S, D)
```

```python
import functools

import jax
import jax.numpy as jnp
import jax.experimental.pallas as pl
import jax.experimental.pallas.tpu as pltpu

_LANES = 128
_B_HEADS = 32
_B_WIN = 8
_B_DIL = 2
_HALO = 16
_MASKED = -1000000000.0
_F32 = jnp.float32
_BF16 = jnp.bfloat16


_DMA_PLAN = {
    "begin": ((), ("bq", "bk", "x0")),
    (0, 0): (("bq", "bk", "x0"), ("bv", "x1", "bwo")),
    (0, 2): (("bv",), (0,)),
    (1, 0): ((), (1,)),
    (2, 0): (("x1", "bwo", 0), (2, 3)),
    (3, 0): ((1,), (4,)),
    (4, 0): ((2,), (5, 6)),
    (5, 0): ((3, 4), (7,)),
    (6, 0): ((5,), ("wo",)),
    (7, 0): ((6,), ()),
    (8, 0): ((7,), ()),
    "wo": (("wo",), ()),
}
_TRANSPOSE_PLAN = {2: (0,), 3: (1,), 4: (2,), 5: (3, 4), 6: (5,), 7: (6,), 8: (7,)}


def _mm(a, b):
    return jax.lax.dot_general(a, b, (((1,), (0,)), ((), ())),
                               preferred_element_type=_F32)


def _mm_nt(a, b):
    return jax.lax.dot_general(a, b, (((1,), (1,)), ((), ())),
                               preferred_element_type=_F32)


def _iota(shape, dim):
    return jax.lax.broadcasted_iota(jnp.int32, shape, dim)


def _step_order(n):
    ops = []
    for p in range(n):
        ops.append(("qk", p, None))
        if p >= 2:
            ops.append(("pv", p - 2, None))
        ops.append(("v", p, None))
        ops.append(("softmax", p, None))
    ops += [("pv", n - 2, None), ("out", 0, 4), ("pv", n - 1, None), ("out", 4, n)]
    return ops


def _kernel(x_hbm, mem0_ref, wq_hbm, wk_hbm, wv_hbm, wo_hbm, bqkv_hbm, bwo_hbm,
            gate_ref, out_hbm,
            x_ref, stage_ref, wt_ref, wo_ref, bqkv_ref, bwo_ref, b32_ref,
            bp_ref, qkv_ref, att_ref, b_ref, g_ref,
            out_ref, in_sem, w_sem, out_sem,
            *, seg, dh, t_chunk, t_sub, group):
    S, D = x_ref.shape
    M = mem0_ref.shape[0]
    L = M + seg
    n_seg = S // seg
    n_pair, pw = wt_ref.shape[0], 2 * dh
    n_chunk = S // t_chunk
    ppc = n_pair // n_chunk
    n_tile = D // _LANES
    bdh = D // _B_HEADS

    x_head = 2 * t_chunk
    cp = {
        "x0": [pltpu.make_async_copy(x_hbm.at[0:x_head], x_ref.at[0:x_head], in_sem.at[0])],
        "x1": [pltpu.make_async_copy(x_hbm.at[x_head:S], x_ref.at[x_head:S], in_sem.at[1])],
        "bwo": [pltpu.make_async_copy(bwo_hbm, bwo_ref, in_sem.at[2])],
        "wo": [pltpu.make_async_copy(wo_hbm, wo_ref, in_sem.at[3])],
    }
    for m, name in enumerate(("bq", "bk", "bv")):
        cols = slice(m * D, (m + 1) * D)
        cp[name] = [pltpu.make_async_copy(bqkv_hbm.at[:, cols], bqkv_ref.at[m],
                                          in_sem.at[4 + m])]
    for c in range(n_chunk):
        rows = slice(c * ppc * pw, (c + 1) * ppc * pw)
        cp[c] = [pltpu.make_async_copy(src.at[rows], stage_ref.at[m, rows], w_sem.at[c, m])
                 for m, src in enumerate((wq_hbm, wk_hbm, wv_hbm))]

    def dma(point):
        waits, starts = _DMA_PLAN.get(point, ((), ()))
        for name in waits:
            for copy in cp[name]:
                copy.wait()
        for name in starts:
            for copy in cp[name]:
                copy.start()

    dma("begin")

    def reorder_rows(m, tile):
        for j in range(n_tile):
            b32_ref[m, j] = tile(j).astype(_F32)
            for d in range(bdh):
                bp_ref[m, d * _B_HEADS:(d + 1) * _B_HEADS, j * _LANES:(j + 1) * _LANES] = (
                    b32_ref[m, j, pl.ds(d, _B_HEADS, stride=bdh), :].astype(_BF16))

    b_scale = float(bdh) ** -0.5

    def b_project(c, m):
        if c == 0:
            reorder_rows(m, lambda j: bqkv_ref[m, j * _LANES:(j + 1) * _LANES, :].T)
        y = _mm_nt(x_ref[c * t_chunk:(c + 1) * t_chunk, :], bp_ref[m])
        if m == 0:
            y = y * b_scale
        for j in range(n_tile):
            cols = slice(j * _LANES, (j + 1) * _LANES)
            qkv_ref[m, j, _HALO + c * t_chunk:_HALO + (c + 1) * t_chunk, :] = y[:, cols]
            if c == 0 and m > 0:
                qkv_ref[m, j, 0:_HALO, :] = jnp.broadcast_to(y[0:1, cols], (_HALO, _LANES))

    def b_attend(r):
        def rows(m, j, w):
            return qkv_ref[m, j, pl.ds(_HALO + r - w * _B_DIL, t_sub), :]

        q = [rows(0, j, 0) for j in range(n_tile)]
        logits = []
        for w in range(_B_WIN):
            s = functools.reduce(jnp.add, [q[j] * rows(1, j, w) for j in range(n_tile)])
            s = s + pltpu.roll(s, 2 * _B_HEADS, 1)
            s = s + pltpu.roll(s, _B_HEADS, 1)
            if r < w * _B_DIL:
                pos = r + _iota((t_sub, _LANES), 0)
                s = jnp.where(pos >= w * _B_DIL, s, _MASKED)
            logits.append(s)
        mx = functools.reduce(jnp.maximum, logits)
        es = [jnp.exp(s - mx) for s in logits]
        inv = 1.0 / functools.reduce(jnp.add, es)
        for j in range(n_tile):
            acc = functools.reduce(jnp.add, [es[w] * rows(2, j, w) for w in range(_B_WIN)])
            att_ref[r:r + t_sub, j * _LANES:(j + 1) * _LANES] = (acc * inv).astype(_BF16)

    def b_output(c):
        if c == 0:
            reorder_rows(3, lambda j: bwo_ref[:, j * _LANES:(j + 1) * _LANES])
        rows = slice(c * t_chunk, (c + 1) * t_chunk)
        g = jax.nn.sigmoid(jnp.sum(x_ref[rows, :].astype(_F32) * gate_ref[...].astype(_F32),
                                   axis=1, keepdims=True))
        g_ref[rows, :] = jnp.broadcast_to(g, (t_chunk, _LANES))
        b_ref[rows, :] = (1.0 - g) * _mm(att_ref[rows, :], bp_ref[3])

    def transpose_w(c, m):
        for p in range(c * ppc, (c + 1) * ppc):
            wt_ref[p, :, m * pw:(m + 1) * pw] = stage_ref[m, p * pw:(p + 1) * pw, :].T

    n_sub = t_chunk // t_sub
    subs = [n_sub * f // 8 for f in (0, 4, 8, 8, 8)]
    for i in range(n_chunk + 2):
        for m in range(4):
            dma((i, m))
            if 1 <= i <= n_chunk:
                for u in range(subs[m], subs[m + 1]):
                    b_attend((i - 1) * t_chunk + u * t_sub)
            if m < 3:
                for c in _TRANSPOSE_PLAN.get(i, ()):
                    transpose_w(c, m)
            if m < 3 and i < n_chunk:
                b_project(i, m)
            if m == 3 and i >= 2:
                b_output(i - 2)

    a_scale = float(dh) ** -0.5

    def seg_rows(s):
        return pl.ds(s * seg if isinstance(s, int) else pl.multiple_of(s * seg, seg), seg)

    def block_diag(t):
        first = _iota((L, pw), 1) < dh
        return jnp.concatenate(
            [jnp.where(first, t, 0.0), jnp.where(first, 0.0, t)], axis=0
        ).astype(_BF16)

    def a_step(s, mem, first_step=False):
        h = jnp.concatenate([mem, x_ref[seg_rows(s), :].astype(_F32)], axis=0)

        row = _iota((L, 2 * L), 0)
        col = _iota((L, 2 * L), 1)
        first = col < L
        key = jnp.where(first, col, col - L)
        visible = (row < M) | (row >= key)

        def softmax(q, kbd):
            sc = jnp.where(visible, _mm_nt(q, kbd) * a_scale, _MASKED)
            m0 = jnp.max(jnp.where(first, sc, -jnp.inf), axis=1, keepdims=True)
            m1 = jnp.max(jnp.where(first, -jnp.inf, sc), axis=1, keepdims=True)
            e = jnp.exp(sc - jnp.where(first, m0, m1))
            s0 = jnp.sum(jnp.where(first, e, 0.0), axis=1, keepdims=True)
            s1 = jnp.sum(jnp.where(first, 0.0, e), axis=1, keepdims=True)
            return e / jnp.where(first, s0, s1)

        def out_proj(p0, p1):
            o = jnp.concatenate([att[p] for p in range(p0, p1)], axis=1)
            return _mm(o, wo_ref[p0 * pw:p1 * pw, :])

        qk, v, prob, att, res = {}, {}, {}, {}, []
        for op, p, p1 in _step_order(n_pair):
            if op == "qk":
                y = _mm(h, wt_ref[p, :, 0:2 * pw])
                qk[p] = y[:, 0:pw], block_diag(y[:, pw:])
            elif op == "v":
                v[p] = block_diag(_mm(h, wt_ref[p, :, 2 * pw:]))
            elif op == "softmax":
                prob[p] = softmax(*qk[p])
            elif op == "pv":
                att[p] = _mm(prob[p], v[p])
            else:
                if first_step and not res:
                    dma("wo")
                res.append(out_proj(p, p1))
        res = functools.reduce(jnp.add, res)
        rows = seg_rows(s)
        g = g_ref[rows, :]
        g = jnp.concatenate([g] * n_tile, axis=1)
        out_ref[rows, :] = (g * res[M:, :] + b_ref[rows, :]).astype(out_ref.dtype)
        return res[0:M, :]

    def cp_out(rows):
        return pltpu.make_async_copy(out_ref.at[rows], out_hbm.at[rows], out_sem.at[0])

    def a_loop(s, mem):
        @pl.when(s % group == 1)
        def _():
            @pl.when(s > 1)
            def _():
                cp_out(pl.ds(pl.multiple_of((s - group) * seg, seg), group * seg)).start()
        return a_step(s, mem)

    mem = a_step(0, mem0_ref[...].astype(_F32), first_step=True)
    cp_out(seg_rows(0)).start()
    jax.lax.fori_loop(1, n_seg, a_loop, mem)
    cp_out(pl.ds((n_seg - group) * seg, group * seg)).start()
    pltpu.make_async_copy(out_ref, out_hbm, out_sem.at[0]).wait()


@functools.partial(jax.jit, static_argnames=("A_seg_len",))
def pallas_gated_mix__memory_aug_recurrent_mem_tr__sliding_local_dilated__prompt_kernel(
    A_x: jax.Array,
    A_mem0: jax.Array,
    A_Wq: jax.Array,
    A_Wk: jax.Array,
    A_Wv: jax.Array,
    A_Wo: jax.Array,
    A_seg_len: int,
    B_x: jax.Array,
    B_wqkv: jax.Array,
    B_wo: jax.Array,
    gate_w: jax.Array,
):
    del B_x
    _, S, D = A_x.shape
    _, H, dh = A_Wq.shape
    M = A_mem0.shape[1]
    seg = int(A_seg_len)
    E = H * dh
    n_pair = H // 2
    t_chunk, t_sub = 256, 128
    group = 9
    assert (S // seg - 1) % group == 0
    n_chunk = S // t_chunk

    def rows_major(w):
        return jnp.transpose(w, (1, 2, 0)).reshape(E, D)

    hbm = pl.BlockSpec(memory_space=pl.ANY)
    vmem = pl.BlockSpec(memory_space=pltpu.VMEM)
    out = pl.pallas_call(
        functools.partial(_kernel, seg=seg, dh=dh, t_chunk=t_chunk, t_sub=t_sub,
                          group=group),
        out_shape=jax.ShapeDtypeStruct((S, D), A_x.dtype),
        in_specs=[hbm, vmem, hbm, hbm, hbm, hbm, hbm, hbm, vmem],
        out_specs=hbm,
        scratch_shapes=[
            pltpu.VMEM((S, D), _BF16),
            pltpu.VMEM((3, E, D), _BF16),
            pltpu.VMEM((n_pair, D, 6 * dh), _BF16),
            pltpu.VMEM((E, D), _BF16),
            pltpu.VMEM((3, D, D), _BF16),
            pltpu.VMEM((D, D), _BF16),
            pltpu.VMEM((4, D // _LANES, D, _LANES), _F32),
            pltpu.VMEM((4, D, D), _BF16),
            pltpu.VMEM((3, D // _LANES, _HALO + S, _LANES), _F32),
            pltpu.VMEM((S, D), _BF16),
            pltpu.VMEM((S, D), _F32),
            pltpu.VMEM((S, _LANES), _F32),
            pltpu.VMEM((S, D), A_x.dtype),
            pltpu.SemaphoreType.DMA((7,)),
            pltpu.SemaphoreType.DMA((n_chunk, 3)),
            pltpu.SemaphoreType.DMA((1,)),
        ],
        compiler_params=pltpu.CompilerParams(vmem_limit_bytes=110 * 1024 * 1024),
    )(A_x.reshape(S, D), A_mem0.reshape(M, D), rows_major(A_Wq), rows_major(A_Wk),
      rows_major(A_Wv), A_Wo.reshape(E, D), B_wqkv, B_wo, gate_w.reshape(1, D))
    return out.reshape(1, S, D)
```

```python
import functools

import jax
import jax.numpy as jnp
import jax.experimental.pallas as pl
import jax.experimental.pallas.tpu as pltpu

_LANES = 128
_B_HEADS = 32
_B_WIN = 8
_B_DIL = 2
_HALO = 16
_MASKED = -1000000000.0
_F32 = jnp.float32
_BF16 = jnp.bfloat16


_DMA_PLAN = {
    "begin": ((), ("bq", "bk", "x0")),
    (0, 0): (("bq", "bk", "x0"), ("bv", "x1", "bwo")),
    (0, 2): (("bv",), (0,)),
    (1, 0): ((), (1,)),
    (2, 0): (("x1", "bwo", 0), (2, 3)),
    (3, 0): ((1,), (4,)),
    (4, 0): ((2,), (5, 6)),
    (5, 0): ((3, 4), (7,)),
    (6, 0): ((5,), ("wo",)),
    (7, 0): ((6,), ()),
    (8, 0): ((7,), ()),
    "wo": (("wo",), ()),
}
_TRANSPOSE_PLAN = {2: (0,), 3: (1,), 4: (2,), 5: (3, 4), 6: (5,), 7: (6,), 8: (7,)}


def _mm(a, b):
    return jax.lax.dot_general(a, b, (((1,), (0,)), ((), ())),
                               preferred_element_type=_F32)


def _mm_nt(a, b):
    return jax.lax.dot_general(a, b, (((1,), (1,)), ((), ())),
                               preferred_element_type=_F32)


def _iota(shape, dim):
    return jax.lax.broadcasted_iota(jnp.int32, shape, dim)


def _step_order(n):
    ops = []
    lag = 3
    for i in range(n + lag + 1):
        for op, p in (("qk", i), ("v", i - lag), ("softmax", i - 1), ("pv", i - lag - 1)):
            if 0 <= p < n:
                ops.append((op, p, None))
    ops.append(("out", 0, n))
    return ops


def _kernel(x_hbm, mem0_ref, wq_hbm, wk_hbm, wv_hbm, wo_hbm, bqkv_hbm, bwo_hbm,
            gate_ref, out_hbm,
            x_ref, stage_ref, wt_ref, wo_ref, bqkv_ref, bwo_ref, b32_ref,
            bp_ref, qkv_ref, att_ref, b_ref, g_ref,
            out_ref, in_sem, w_sem, out_sem,
            *, seg, dh, t_chunk, t_sub, group):
    S, D = x_ref.shape
    M = mem0_ref.shape[0]
    L = M + seg
    n_seg = S // seg
    n_pair, pw = wt_ref.shape[0], 2 * dh
    n_chunk = S // t_chunk
    ppc = n_pair // n_chunk
    n_tile = D // _LANES
    bdh = D // _B_HEADS

    x_head = 2 * t_chunk
    cp = {
        "x0": [pltpu.make_async_copy(x_hbm.at[0:x_head], x_ref.at[0:x_head], in_sem.at[0])],
        "x1": [pltpu.make_async_copy(x_hbm.at[x_head:S], x_ref.at[x_head:S], in_sem.at[1])],
        "bwo": [pltpu.make_async_copy(bwo_hbm, bwo_ref, in_sem.at[2])],
        "wo": [pltpu.make_async_copy(wo_hbm, wo_ref, in_sem.at[3])],
    }
    for m, name in enumerate(("bq", "bk", "bv")):
        cols = slice(m * D, (m + 1) * D)
        cp[name] = [pltpu.make_async_copy(bqkv_hbm.at[:, cols], bqkv_ref.at[m],
                                          in_sem.at[4 + m])]
    for c in range(n_chunk):
        rows = slice(c * ppc * pw, (c + 1) * ppc * pw)
        cp[c] = [pltpu.make_async_copy(src.at[rows], stage_ref.at[m, rows], w_sem.at[c, m])
                 for m, src in enumerate((wq_hbm, wk_hbm, wv_hbm))]

    def dma(point):
        waits, starts = _DMA_PLAN.get(point, ((), ()))
        for name in waits:
            for copy in cp[name]:
                copy.wait()
        for name in starts:
            for copy in cp[name]:
                copy.start()

    dma("begin")

    def reorder_rows(m, tile):
        for j in range(n_tile):
            b32_ref[m, j] = tile(j).astype(_F32)
            for d in range(bdh):
                bp_ref[m, d * _B_HEADS:(d + 1) * _B_HEADS, j * _LANES:(j + 1) * _LANES] = (
                    b32_ref[m, j, pl.ds(d, _B_HEADS, stride=bdh), :].astype(_BF16))

    b_scale = float(bdh) ** -0.5

    def b_project(c, m):
        if c == 0:
            reorder_rows(m, lambda j: bqkv_ref[m, j * _LANES:(j + 1) * _LANES, :].T)
        y = _mm_nt(x_ref[c * t_chunk:(c + 1) * t_chunk, :], bp_ref[m])
        if m == 0:
            y = y * b_scale
        for j in range(n_tile):
            cols = slice(j * _LANES, (j + 1) * _LANES)
            qkv_ref[m, j, _HALO + c * t_chunk:_HALO + (c + 1) * t_chunk, :] = y[:, cols]
            if c == 0 and m > 0:
                qkv_ref[m, j, 0:_HALO, :] = jnp.broadcast_to(y[0:1, cols], (_HALO, _LANES))

    def b_attend(r):
        def rows(m, j, w):
            return qkv_ref[m, j, pl.ds(_HALO + r - w * _B_DIL, t_sub), :]

        q = [rows(0, j, 0) for j in range(n_tile)]
        logits = []
        for w in range(_B_WIN):
            s = functools.reduce(jnp.add, [q[j] * rows(1, j, w) for j in range(n_tile)])
            s = s + pltpu.roll(s, 2 * _B_HEADS, 1)
            s = s + pltpu.roll(s, _B_HEADS, 1)
            if r < w * _B_DIL:
                pos = r + _iota((t_sub, _LANES), 0)
                s = jnp.where(pos >= w * _B_DIL, s, _MASKED)
            logits.append(s)
        mx = functools.reduce(jnp.maximum, logits)
        es = [jnp.exp(s - mx) for s in logits]
        inv = 1.0 / functools.reduce(jnp.add, es)
        for j in range(n_tile):
            acc = functools.reduce(jnp.add, [es[w] * rows(2, j, w) for w in range(_B_WIN)])
            att_ref[r:r + t_sub, j * _LANES:(j + 1) * _LANES] = (acc * inv).astype(_BF16)

    def b_output(c):
        if c == 0:
            reorder_rows(3, lambda j: bwo_ref[:, j * _LANES:(j + 1) * _LANES])
        rows = slice(c * t_chunk, (c + 1) * t_chunk)
        g = jax.nn.sigmoid(jnp.sum(x_ref[rows, :].astype(_F32) * gate_ref[...].astype(_F32),
                                   axis=1, keepdims=True))
        g_ref[rows, :] = jnp.broadcast_to(g, (t_chunk, _LANES))
        b_ref[rows, :] = (1.0 - g) * _mm(att_ref[rows, :], bp_ref[3])

    def transpose_w(c, m):
        for p in range(c * ppc, (c + 1) * ppc):
            wt_ref[p, :, m * pw:(m + 1) * pw] = stage_ref[m, p * pw:(p + 1) * pw, :].T

    n_sub = t_chunk // t_sub
    subs = [n_sub * f // 8 for f in (0, 4, 8, 8, 8)]
    for i in range(n_chunk + 2):
        for m in range(4):
            dma((i, m))
            if 1 <= i <= n_chunk:
                for u in range(subs[m], subs[m + 1]):
                    b_attend((i - 1) * t_chunk + u * t_sub)
            if m < 3:
                for c in _TRANSPOSE_PLAN.get(i, ()):
                    transpose_w(c, m)
            if m < 3 and i < n_chunk:
                b_project(i, m)
            if m == 3 and i >= 2:
                b_output(i - 2)

    a_scale = float(dh) ** -0.5

    def seg_rows(s):
        return pl.ds(s * seg if isinstance(s, int) else pl.multiple_of(s * seg, seg), seg)

    def block_diag(t):
        first = _iota((L, pw), 1) < dh
        return jnp.concatenate(
            [jnp.where(first, t, 0.0), jnp.where(first, 0.0, t)], axis=0
        ).astype(_BF16)

    def a_step(s, mem, first_step=False):
        h = jnp.concatenate([mem, x_ref[seg_rows(s), :].astype(_F32)], axis=0)

        row = _iota((L, 2 * L), 0)
        col = _iota((L, 2 * L), 1)
        first = col < L
        key = jnp.where(first, col, col - L)
        visible = (row < M) | (row >= key)

        def softmax(q, kbd):
            sc = jnp.where(visible, _mm_nt(q, kbd) * a_scale, _MASKED)
            m0 = jnp.max(jnp.where(first, sc, -jnp.inf), axis=1, keepdims=True)
            m1 = jnp.max(jnp.where(first, -jnp.inf, sc), axis=1, keepdims=True)
            e = jnp.exp(sc - jnp.where(first, m0, m1))
            s0 = jnp.sum(jnp.where(first, e, 0.0), axis=1, keepdims=True)
            s1 = jnp.sum(jnp.where(first, 0.0, e), axis=1, keepdims=True)
            return e / jnp.where(first, s0, s1)

        def out_proj(p0, p1):
            o = jnp.concatenate([att[p] for p in range(p0, p1)], axis=1)
            return _mm(o, wo_ref[p0 * pw:p1 * pw, :])

        qk, v, prob, att, res = {}, {}, {}, {}, []
        for op, p, p1 in _step_order(n_pair):
            if op == "qk":
                y = _mm(h, wt_ref[p, :, 0:2 * pw])
                qk[p] = y[:, 0:pw], block_diag(y[:, pw:])
            elif op == "v":
                v[p] = block_diag(_mm(h, wt_ref[p, :, 2 * pw:]))
            elif op == "softmax":
                prob[p] = softmax(*qk[p])
            elif op == "pv":
                att[p] = _mm(prob[p], v[p])
            else:
                if first_step and not res:
                    dma("wo")
                res.append(out_proj(p, p1))
        res = functools.reduce(jnp.add, res)
        rows = seg_rows(s)
        g = g_ref[rows, :]
        g = jnp.concatenate([g] * n_tile, axis=1)
        out_ref[rows, :] = (g * res[M:, :] + b_ref[rows, :]).astype(out_ref.dtype)
        return res[0:M, :]

    def cp_out(rows):
        return pltpu.make_async_copy(out_ref.at[rows], out_hbm.at[rows], out_sem.at[0])

    def a_loop(s, mem):
        @pl.when(s % group == 1)
        def _():
            @pl.when(s > 1)
            def _():
                cp_out(pl.ds(pl.multiple_of((s - group) * seg, seg), group * seg)).start()
        return a_step(s, mem)

    mem = a_step(0, mem0_ref[...].astype(_F32), first_step=True)
    cp_out(seg_rows(0)).start()
    jax.lax.fori_loop(1, n_seg, a_loop, mem)
    cp_out(pl.ds((n_seg - group) * seg, group * seg)).start()
    pltpu.make_async_copy(out_ref, out_hbm, out_sem.at[0]).wait()


@functools.partial(jax.jit, static_argnames=("A_seg_len",))
def pallas_gated_mix__memory_aug_recurrent_mem_tr__sliding_local_dilated__prompt_kernel(
    A_x: jax.Array,
    A_mem0: jax.Array,
    A_Wq: jax.Array,
    A_Wk: jax.Array,
    A_Wv: jax.Array,
    A_Wo: jax.Array,
    A_seg_len: int,
    B_x: jax.Array,
    B_wqkv: jax.Array,
    B_wo: jax.Array,
    gate_w: jax.Array,
):
    del B_x
    _, S, D = A_x.shape
    _, H, dh = A_Wq.shape
    M = A_mem0.shape[1]
    seg = int(A_seg_len)
    E = H * dh
    n_pair = H // 2
    t_chunk, t_sub = 256, 128
    group = 9
    assert (S // seg - 1) % group == 0
    n_chunk = S // t_chunk

    def rows_major(w):
        return jnp.transpose(w, (1, 2, 0)).reshape(E, D)

    hbm = pl.BlockSpec(memory_space=pl.ANY)
    vmem = pl.BlockSpec(memory_space=pltpu.VMEM)
    out = pl.pallas_call(
        functools.partial(_kernel, seg=seg, dh=dh, t_chunk=t_chunk, t_sub=t_sub,
                          group=group),
        out_shape=jax.ShapeDtypeStruct((S, D), A_x.dtype),
        in_specs=[hbm, vmem, hbm, hbm, hbm, hbm, hbm, hbm, vmem],
        out_specs=hbm,
        scratch_shapes=[
            pltpu.VMEM((S, D), _BF16),
            pltpu.VMEM((3, E, D), _BF16),
            pltpu.VMEM((n_pair, D, 6 * dh), _BF16),
            pltpu.VMEM((E, D), _BF16),
            pltpu.VMEM((3, D, D), _BF16),
            pltpu.VMEM((D, D), _BF16),
            pltpu.VMEM((4, D // _LANES, D, _LANES), _F32),
            pltpu.VMEM((4, D, D), _BF16),
            pltpu.VMEM((3, D // _LANES, _HALO + S, _LANES), _F32),
            pltpu.VMEM((S, D), _BF16),
            pltpu.VMEM((S, D), _F32),
            pltpu.VMEM((S, _LANES), _F32),
            pltpu.VMEM((S, D), A_x.dtype),
            pltpu.SemaphoreType.DMA((7,)),
            pltpu.SemaphoreType.DMA((n_chunk, 3)),
            pltpu.SemaphoreType.DMA((1,)),
        ],
        compiler_params=pltpu.CompilerParams(vmem_limit_bytes=110 * 1024 * 1024),
    )(A_x.reshape(S, D), A_mem0.reshape(M, D), rows_major(A_Wq), rows_major(A_Wk),
      rows_major(A_Wv), A_Wo.reshape(E, D), B_wqkv, B_wo, gate_w.reshape(1, D))
    return out.reshape(1, S, D)
```

```python
import functools

import jax
import jax.numpy as jnp
import jax.experimental.pallas as pl
import jax.experimental.pallas.tpu as pltpu

_LANES = 128
_B_HEADS = 32
_B_WIN = 8
_B_DIL = 2
_HALO = 16
_MASKED = -1000000000.0
_F32 = jnp.float32
_BF16 = jnp.bfloat16


_DMA_PLAN = {
    "begin": ((), ("bq", "bk", "x0")),
    (0, 0): (("bq", "bk", "x0"), ("bv", "x1", "bwo")),
    (0, 2): (("bv",), (0,)),
    (1, 0): ((), (1,)),
    (2, 0): (("x1", "bwo", 0), (2, 3)),
    (3, 0): ((1,), (4,)),
    (4, 0): ((2,), (5,)),
    (5, 0): ((3,), (6,)),
    (6, 0): ((4,), (7,)),
    (7, 0): ((5,), ("wo",)),
    (8, 0): ((6, 7), ()),
    "wo": (("wo",), ()),
}
_TRANSPOSE_PLAN = {2: (0,), 3: (1,), 4: (2,), 5: (3,), 6: (4,), 7: (5,), 8: (6, 7)}


def _mm(a, b):
    return jax.lax.dot_general(a, b, (((1,), (0,)), ((), ())),
                               preferred_element_type=_F32)


def _mm_nt(a, b):
    return jax.lax.dot_general(a, b, (((1,), (1,)), ((), ())),
                               preferred_element_type=_F32)


def _iota(shape, dim):
    return jax.lax.broadcasted_iota(jnp.int32, shape, dim)


def _step_order(n):
    ops = []
    lag = 3
    for i in range(n + lag + 1):
        for op, p in (("qk", i), ("softmax", i - 1), ("v", i - lag), ("pv", i - lag - 1)):
            if 0 <= p < n:
                ops.append((op, p, None))
    ops.append(("out", 0, n))
    return ops


def _kernel(x_hbm, mem0_ref, wq_hbm, wk_hbm, wv_hbm, wo_hbm, bqkv_hbm, bwo_hbm,
            gate_ref, out_hbm,
            x_ref, stage_ref, wt_ref, wo_ref, bqkv_ref, bwo_ref, b32_ref,
            bp_ref, qkv_ref, att_ref, b_ref, g_ref,
            out_ref, in_sem, w_sem, out_sem,
            *, seg, dh, t_chunk, t_sub, group):
    S, D = x_ref.shape
    M = mem0_ref.shape[0]
    L = M + seg
    n_seg = S // seg
    n_pair, pw = wt_ref.shape[0], 2 * dh
    n_chunk = S // t_chunk
    ppc = n_pair // n_chunk
    n_tile = D // _LANES
    bdh = D // _B_HEADS

    x_head = 2 * t_chunk
    cp = {
        "x0": [pltpu.make_async_copy(x_hbm.at[0:x_head], x_ref.at[0:x_head], in_sem.at[0])],
        "x1": [pltpu.make_async_copy(x_hbm.at[x_head:S], x_ref.at[x_head:S], in_sem.at[1])],
        "bwo": [pltpu.make_async_copy(bwo_hbm, bwo_ref, in_sem.at[2])],
        "wo": [pltpu.make_async_copy(wo_hbm, wo_ref, in_sem.at[3])],
    }
    for m, name in enumerate(("bq", "bk", "bv")):
        cols = slice(m * D, (m + 1) * D)
        cp[name] = [pltpu.make_async_copy(bqkv_hbm.at[:, cols], bqkv_ref.at[m],
                                          in_sem.at[4 + m])]
    for c in range(n_chunk):
        rows = slice(c * ppc * pw, (c + 1) * ppc * pw)
        cp[c] = [pltpu.make_async_copy(src.at[rows], stage_ref.at[m, rows], w_sem.at[c, m])
                 for m, src in enumerate((wq_hbm, wk_hbm, wv_hbm))]

    def dma(point):
        waits, starts = _DMA_PLAN.get(point, ((), ()))
        for name in waits:
            for copy in cp[name]:
                copy.wait()
        for name in starts:
            for copy in cp[name]:
                copy.start()

    dma("begin")

    def reorder_rows(m, tile):
        for j in range(n_tile):
            b32_ref[m, j] = tile(j).astype(_F32)
            for d in range(bdh):
                bp_ref[m, d * _B_HEADS:(d + 1) * _B_HEADS, j * _LANES:(j + 1) * _LANES] = (
                    b32_ref[m, j, pl.ds(d, _B_HEADS, stride=bdh), :].astype(_BF16))

    b_scale = float(bdh) ** -0.5

    def b_project(c, m):
        if c == 0:
            reorder_rows(m, lambda j: bqkv_ref[m, j * _LANES:(j + 1) * _LANES, :].T)
        y = _mm_nt(x_ref[c * t_chunk:(c + 1) * t_chunk, :], bp_ref[m])
        if m == 0:
            y = y * b_scale
        for j in range(n_tile):
            cols = slice(j * _LANES, (j + 1) * _LANES)
            qkv_ref[m, j, _HALO + c * t_chunk:_HALO + (c + 1) * t_chunk, :] = y[:, cols]
            if c == 0 and m > 0:
                qkv_ref[m, j, 0:_HALO, :] = jnp.broadcast_to(y[0:1, cols], (_HALO, _LANES))

    def b_attend(r):
        def rows(m, j, w):
            return qkv_ref[m, j, pl.ds(_HALO + r - w * _B_DIL, t_sub), :]

        q = [rows(0, j, 0) for j in range(n_tile)]
        logits = []
        for w in range(_B_WIN):
            s = functools.reduce(jnp.add, [q[j] * rows(1, j, w) for j in range(n_tile)])
            s = s + pltpu.roll(s, 2 * _B_HEADS, 1)
            s = s + pltpu.roll(s, _B_HEADS, 1)
            if r < w * _B_DIL:
                pos = r + _iota((t_sub, _LANES), 0)
                s = jnp.where(pos >= w * _B_DIL, s, _MASKED)
            logits.append(s)
        mx = functools.reduce(jnp.maximum, logits)
        es = [jnp.exp(s - mx) for s in logits]
        inv = 1.0 / functools.reduce(jnp.add, es)
        for j in range(n_tile):
            acc = functools.reduce(jnp.add, [es[w] * rows(2, j, w) for w in range(_B_WIN)])
            att_ref[r:r + t_sub, j * _LANES:(j + 1) * _LANES] = (acc * inv).astype(_BF16)

    def b_output(c):
        if c == 0:
            reorder_rows(3, lambda j: bwo_ref[:, j * _LANES:(j + 1) * _LANES])
        rows = slice(c * t_chunk, (c + 1) * t_chunk)
        g = jax.nn.sigmoid(jnp.sum(x_ref[rows, :].astype(_F32) * gate_ref[...].astype(_F32).reshape(1, D),
                                   axis=1, keepdims=True))
        g_ref[rows, :] = jnp.broadcast_to(g, (t_chunk, _LANES))
        b_ref[rows, :] = (1.0 - g) * _mm(att_ref[rows, :], bp_ref[3])

    def transpose_w(c, m):
        for p in range(c * ppc, (c + 1) * ppc):
            wt_ref[p, :, m * pw:(m + 1) * pw] = stage_ref[m, p * pw:(p + 1) * pw, :].T

    n_sub = t_chunk // t_sub
    subs = [n_sub * f // 8 for f in (0, 4, 8, 8, 8)]
    for i in range(n_chunk):
        for m in range(4):
            dma((i, m))
            if i >= 1:
                for u in range(subs[m], subs[m + 1]):
                    b_attend((i - 1) * t_chunk + u * t_sub)
            if m < 3:
                for c in _TRANSPOSE_PLAN.get(i, ()):
                    transpose_w(c, m)
            if m < 3:
                b_project(i, m)
            if m == 3 and i >= 2:
                b_output(i - 2)

    dma((n_chunk, 0))
    leftover = [functools.partial(b_attend, r) for r in range(S - t_chunk, S, t_sub)]
    leftover += [functools.partial(transpose_w, c, m)
                 for c in _TRANSPOSE_PLAN[n_chunk] for m in range(3)]
    leftover += [functools.partial(b_output, c) for c in (n_chunk - 2, n_chunk - 1)]

    a_scale = float(dh) ** -0.5

    def seg_rows(s):
        return pl.ds(s * seg if isinstance(s, int) else pl.multiple_of(s * seg, seg), seg)

    def block_diag(t):
        first = _iota((L, pw), 1) < dh
        return jnp.concatenate(
            [jnp.where(first, t, 0.0), jnp.where(first, 0.0, t)], axis=0
        ).astype(_BF16)

    def a_step(s, mem, first_step=False):
        h = jnp.concatenate([mem, x_ref[seg_rows(s), :].astype(_F32)], axis=0)

        row = _iota((L, 2 * L), 0)
        col = _iota((L, 2 * L), 1)
        first = col < L
        key = jnp.where(first, col, col - L)
        visible = (row < M) | (row >= key)

        def softmax(q, kbd):
            sc = jnp.where(visible, _mm_nt(q, kbd) * a_scale, _MASKED)
            m0 = jnp.max(jnp.where(first, sc, -jnp.inf), axis=1, keepdims=True)
            m1 = jnp.max(jnp.where(first, -jnp.inf, sc), axis=1, keepdims=True)
            e = jnp.exp(sc - jnp.where(first, m0, m1))
            s0 = jnp.sum(jnp.where(first, e, 0.0), axis=1, keepdims=True)
            s1 = jnp.sum(jnp.where(first, 0.0, e), axis=1, keepdims=True)
            return e / jnp.where(first, s0, s1)

        def out_proj(p0, p1):
            o = jnp.concatenate([att[p] for p in range(p0, p1)], axis=1)
            return _mm(o, wo_ref[p0 * pw:p1 * pw, :])

        qk, v, prob, att, res = {}, {}, {}, {}, []
        for op, p, p1 in _step_order(n_pair):
            if op == "qk":
                if first_step and p < len(leftover):
                    leftover[p]()
                y = _mm(h, wt_ref[p, :, 0:2 * pw])
                qk[p] = y[:, 0:pw], block_diag(y[:, pw:])
            elif op == "v":
                v[p] = block_diag(_mm(h, wt_ref[p, :, 2 * pw:]))
            elif op == "softmax":
                prob[p] = softmax(*qk[p])
            elif op == "pv":
                att[p] = _mm(prob[p], v[p])
            else:
                if first_step and not res:
                    dma("wo")
                res.append(out_proj(p, p1))
        res = functools.reduce(jnp.add, res)
        rows = seg_rows(s)
        g = g_ref[rows, :]
        g = jnp.concatenate([g] * n_tile, axis=1)
        out_ref[rows, :] = (g * res[M:, :] + b_ref[rows, :]).astype(out_ref.dtype)
        return res[0:M, :]

    def cp_out(rows):
        return pltpu.make_async_copy(out_ref.at[rows], out_hbm.at[rows], out_sem.at[0])

    def a_loop(s, mem):
        @pl.when(s % group == 1)
        def _():
            @pl.when(s > 1)
            def _():
                cp_out(pl.ds(pl.multiple_of((s - group) * seg, seg), group * seg)).start()
        return a_step(s, mem)

    mem = a_step(0, mem0_ref[...].astype(_F32), first_step=True)
    cp_out(seg_rows(0)).start()
    jax.lax.fori_loop(1, n_seg, a_loop, mem)
    cp_out(pl.ds((n_seg - group) * seg, group * seg)).start()
    pltpu.make_async_copy(out_ref, out_hbm, out_sem.at[0]).wait()


@functools.partial(jax.jit, static_argnames=("A_seg_len",))
def pallas_gated_mix__memory_aug_recurrent_mem_tr__sliding_local_dilated__prompt_kernel(
    A_x: jax.Array,
    A_mem0: jax.Array,
    A_Wq: jax.Array,
    A_Wk: jax.Array,
    A_Wv: jax.Array,
    A_Wo: jax.Array,
    A_seg_len: int,
    B_x: jax.Array,
    B_wqkv: jax.Array,
    B_wo: jax.Array,
    gate_w: jax.Array,
):
    del B_x
    _, S, D = A_x.shape
    _, H, dh = A_Wq.shape
    M = A_mem0.shape[1]
    seg = int(A_seg_len)
    E = H * dh
    n_pair = H // 2
    t_chunk, t_sub = 256, 128
    group = 9
    assert (S // seg - 1) % group == 0
    n_chunk = S // t_chunk

    def rows_major(w):
        return jnp.transpose(w, (1, 2, 0)).reshape(E, D)

    hbm = pl.BlockSpec(memory_space=pl.ANY)
    vmem = pl.BlockSpec(memory_space=pltpu.VMEM)
    out = pl.pallas_call(
        functools.partial(_kernel, seg=seg, dh=dh, t_chunk=t_chunk, t_sub=t_sub,
                          group=group),
        out_shape=jax.ShapeDtypeStruct((S, D), A_x.dtype),
        in_specs=[hbm, vmem, hbm, hbm, hbm, hbm, hbm, hbm, vmem],
        out_specs=hbm,
        scratch_shapes=[
            pltpu.VMEM((S, D), _BF16),
            pltpu.VMEM((3, E, D), _BF16),
            pltpu.VMEM((n_pair, D, 6 * dh), _BF16),
            pltpu.VMEM((E, D), _BF16),
            pltpu.VMEM((3, D, D), _BF16),
            pltpu.VMEM((D, D), _BF16),
            pltpu.VMEM((4, D // _LANES, D, _LANES), _F32),
            pltpu.VMEM((4, D, D), _BF16),
            pltpu.VMEM((3, D // _LANES, _HALO + S, _LANES), _F32),
            pltpu.VMEM((S, D), _BF16),
            pltpu.VMEM((S, D), _F32),
            pltpu.VMEM((S, _LANES), _F32),
            pltpu.VMEM((S, D), A_x.dtype),
            pltpu.SemaphoreType.DMA((7,)),
            pltpu.SemaphoreType.DMA((n_chunk, 3)),
            pltpu.SemaphoreType.DMA((1,)),
        ],
        compiler_params=pltpu.CompilerParams(vmem_limit_bytes=110 * 1024 * 1024),
    )(A_x.reshape(S, D), A_mem0.reshape(M, D), rows_major(A_Wq), rows_major(A_Wk),
      rows_major(A_Wv), A_Wo.reshape(E, D), B_wqkv, B_wo, gate_w)
    return out.reshape(1, S, D)
```

```python
import functools

import jax
import jax.numpy as jnp
import jax.experimental.pallas as pl
import jax.experimental.pallas.tpu as pltpu

_LANES = 128
_B_HEADS = 32
_B_WIN = 8
_B_DIL = 2
_HALO = 16
_MASKED = -1000000000.0
_F32 = jnp.float32
_BF16 = jnp.bfloat16


_DMA_PLAN = {
    "begin": ((), ("bq", "bk", "x0")),
    (0, 0): (("bq", "bk", "x0"), ("bv", "x1", "bwo")),
    (0, 2): (("bv",), (0,)),
    (1, 0): ((), (1,)),
    (2, 0): (("x1", "bwo", 0), (2, 3)),
    (3, 0): ((1,), (4,)),
    (4, 0): ((2,), (5,)),
    (5, 0): ((3,), (6,)),
    (6, 0): ((4,), (7,)),
    (7, 0): ((5,), ("wo",)),
    (8, 0): ((6, 7), ()),
    "wo": (("wo",), ()),
}
_TRANSPOSE_PLAN = {2: (0,), 3: (1,), 4: (2,), 5: (3,), 6: (4,), 7: (5,), 8: (6, 7)}


def _mm(a, b):
    return jax.lax.dot_general(a, b, (((1,), (0,)), ((), ())),
                               preferred_element_type=_F32)


def _mm_nt(a, b):
    return jax.lax.dot_general(a, b, (((1,), (1,)), ((), ())),
                               preferred_element_type=_F32)


def _iota(shape, dim):
    return jax.lax.broadcasted_iota(jnp.int32, shape, dim)


def _step_order(n):
    ops = []
    lags = (("qk", 0), ("softmax", 1), ("v", 3), ("pv", 9))
    for i in range(n + lags[-1][1]):
        ops += [(op, i - lag) for op, lag in lags if 0 <= i - lag < n]
    return ops


def _kernel(x_hbm, mem0_ref, wq_hbm, wk_hbm, wv_hbm, wo_hbm, bqkv_hbm, bwo_hbm,
            gate_ref, out_hbm,
            x_ref, stage_ref, wt_ref, wo_ref, bqkv_ref, bwo_ref, b32_ref,
            bp_ref, qkv_ref, att_ref, b_ref, g_ref,
            out_ref, in_sem, w_sem, out_sem,
            *, seg, dh, t_chunk, t_sub, group):
    S, D = x_ref.shape
    M = mem0_ref.shape[0]
    L = M + seg
    n_seg = S // seg
    n_pair, pw = wt_ref.shape[0], 2 * dh
    n_chunk = S // t_chunk
    ppc = n_pair // n_chunk
    n_tile = D // _LANES
    bdh = D // _B_HEADS

    x_head = 2 * t_chunk
    cp = {
        "x0": [pltpu.make_async_copy(x_hbm.at[0:x_head], x_ref.at[0:x_head], in_sem.at[0])],
        "x1": [pltpu.make_async_copy(x_hbm.at[x_head:S], x_ref.at[x_head:S], in_sem.at[1])],
        "bwo": [pltpu.make_async_copy(bwo_hbm, bwo_ref, in_sem.at[2])],
        "wo": [pltpu.make_async_copy(wo_hbm, wo_ref, in_sem.at[3])],
    }
    for m, name in enumerate(("bq", "bk", "bv")):
        cols = slice(m * D, (m + 1) * D)
        cp[name] = [pltpu.make_async_copy(bqkv_hbm.at[:, cols], bqkv_ref.at[m],
                                          in_sem.at[4 + m])]
    for c in range(n_chunk):
        rows = slice(c * ppc * pw, (c + 1) * ppc * pw)
        cp[c] = [pltpu.make_async_copy(src.at[rows], stage_ref.at[m, rows], w_sem.at[c, m])
                 for m, src in enumerate((wq_hbm, wk_hbm, wv_hbm))]

    def dma(point):
        waits, starts = _DMA_PLAN.get(point, ((), ()))
        for name in waits:
            for copy in cp[name]:
                copy.wait()
        for name in starts:
            for copy in cp[name]:
                copy.start()

    dma("begin")

    def reorder_rows(m, tile):
        for j in range(n_tile):
            b32_ref[m, j] = tile(j).astype(_F32)
            for d in range(bdh):
                bp_ref[m, d * _B_HEADS:(d + 1) * _B_HEADS, j * _LANES:(j + 1) * _LANES] = (
                    b32_ref[m, j, pl.ds(d, _B_HEADS, stride=bdh), :].astype(_BF16))

    b_scale = float(bdh) ** -0.5

    def b_project(c, m):
        if c == 0:
            reorder_rows(m, lambda j: bqkv_ref[m, j * _LANES:(j + 1) * _LANES, :].T)
        y = _mm_nt(x_ref[c * t_chunk:(c + 1) * t_chunk, :], bp_ref[m])
        if m == 0:
            y = y * b_scale
        for j in range(n_tile):
            cols = slice(j * _LANES, (j + 1) * _LANES)
            qkv_ref[m, j, _HALO + c * t_chunk:_HALO + (c + 1) * t_chunk, :] = y[:, cols]
            if c == 0 and m > 0:
                qkv_ref[m, j, 0:_HALO, :] = jnp.broadcast_to(y[0:1, cols], (_HALO, _LANES))

    def b_attend(r):
        def rows(m, j, w):
            return qkv_ref[m, j, pl.ds(_HALO + r - w * _B_DIL, t_sub), :]

        q = [rows(0, j, 0) for j in range(n_tile)]
        logits = []
        for w in range(_B_WIN):
            s = functools.reduce(jnp.add, [q[j] * rows(1, j, w) for j in range(n_tile)])
            s = s + pltpu.roll(s, 2 * _B_HEADS, 1)
            s = s + pltpu.roll(s, _B_HEADS, 1)
            if r < w * _B_DIL:
                pos = r + _iota((t_sub, _LANES), 0)
                s = jnp.where(pos >= w * _B_DIL, s, _MASKED)
            logits.append(s)
        mx = functools.reduce(jnp.maximum, logits)
        es = [jnp.exp(s - mx) for s in logits]
        inv = 1.0 / functools.reduce(jnp.add, es)
        for j in range(n_tile):
            acc = functools.reduce(jnp.add, [es[w] * rows(2, j, w) for w in range(_B_WIN)])
            att_ref[r:r + t_sub, j * _LANES:(j + 1) * _LANES] = (acc * inv).astype(_BF16)

    def b_output(c):
        if c == 0:
            reorder_rows(3, lambda j: bwo_ref[:, j * _LANES:(j + 1) * _LANES])
        rows = slice(c * t_chunk, (c + 1) * t_chunk)
        g = jax.nn.sigmoid(jnp.sum(x_ref[rows, :].astype(_F32) * gate_ref[...].astype(_F32).reshape(1, D),
                                   axis=1, keepdims=True))
        g_ref[rows, :] = jnp.broadcast_to(g, (t_chunk, _LANES))
        b_ref[rows, :] = (1.0 - g) * _mm(att_ref[rows, :], bp_ref[3])

    def transpose_w(c, m):
        for p in range(c * ppc, (c + 1) * ppc):
            wt_ref[p, :, m * pw:(m + 1) * pw] = stage_ref[m, p * pw:(p + 1) * pw, :].T

    n_sub = t_chunk // t_sub
    subs = [n_sub * f // 8 for f in (0, 4, 8, 8, 8)]
    for i in range(n_chunk):
        for m in range(4):
            dma((i, m))
            if i >= 1:
                for u in range(subs[m], subs[m + 1]):
                    b_attend((i - 1) * t_chunk + u * t_sub)
            if m < 3:
                for c in _TRANSPOSE_PLAN.get(i, ()):
                    transpose_w(c, m)
            if m < 3:
                b_project(i, m)
            if m == 3 and i >= 2:
                b_output(i - 2)

    dma((n_chunk, 0))
    leftover = [functools.partial(b_attend, r) for r in range(S - t_chunk, S, t_sub)]
    leftover += [functools.partial(transpose_w, c, m)
                 for c in _TRANSPOSE_PLAN[n_chunk] for m in range(3)]
    leftover += [functools.partial(b_output, c) for c in (n_chunk - 2, n_chunk - 1)]

    a_scale = float(dh) ** -0.5

    def seg_rows(s):
        return pl.ds(s * seg if isinstance(s, int) else pl.multiple_of(s * seg, seg), seg)

    def block_diag(t):
        first = _iota((L, pw), 1) < dh
        return jnp.concatenate(
            [jnp.where(first, t, 0.0), jnp.where(first, 0.0, t)], axis=0
        ).astype(_BF16)

    def a_step(s, mem, first_step=False):
        h = jnp.concatenate([mem, x_ref[seg_rows(s), :].astype(_F32)], axis=0)

        row = _iota((L, 2 * L), 0)
        col = _iota((L, 2 * L), 1)
        first = col < L
        key = jnp.where(first, col, col - L)
        visible = (row < M) | (row >= key)

        def softmax(q, kbd):
            sc = jnp.where(visible, _mm_nt(q, kbd) * a_scale, _MASKED)
            m0 = jnp.max(jnp.where(first, sc, -jnp.inf), axis=1, keepdims=True)
            m1 = jnp.max(jnp.where(first, -jnp.inf, sc), axis=1, keepdims=True)
            e = jnp.exp(sc - jnp.where(first, m0, m1))
            s0 = jnp.sum(jnp.where(first, e, 0.0), axis=1, keepdims=True)
            s1 = jnp.sum(jnp.where(first, 0.0, e), axis=1, keepdims=True)
            return e / jnp.where(first, s0, s1)

        qk, v, prob, att = {}, {}, {}, {}
        for op, p in _step_order(n_pair):
            if op == "qk":
                if first_step and p < len(leftover):
                    leftover[p]()
                y = _mm(h, wt_ref[p, :, 0:2 * pw])
                qk[p] = y[:, 0:pw], block_diag(y[:, pw:])
            elif op == "v":
                v[p] = block_diag(_mm(h, wt_ref[p, :, 2 * pw:]))
            elif op == "softmax":
                prob[p] = softmax(*qk[p])
            else:
                att[p] = _mm(prob[p], v[p])
        if first_step:
            dma("wo")
        res = _mm(jnp.concatenate([att[p] for p in range(n_pair)], axis=1), wo_ref[...])
        rows = seg_rows(s)
        g = g_ref[rows, :]
        g = jnp.concatenate([g] * n_tile, axis=1)
        out_ref[rows, :] = (g * res[M:, :] + b_ref[rows, :]).astype(out_ref.dtype)
        return res[0:M, :]

    def cp_out(rows):
        return pltpu.make_async_copy(out_ref.at[rows], out_hbm.at[rows], out_sem.at[0])

    def a_loop(s, mem):
        @pl.when(s % group == 1)
        def _():
            @pl.when(s > 1)
            def _():
                cp_out(pl.ds(pl.multiple_of((s - group) * seg, seg), group * seg)).start()
        return a_step(s, mem)

    mem = a_step(0, mem0_ref[...].astype(_F32), first_step=True)
    cp_out(seg_rows(0)).start()
    jax.lax.fori_loop(1, n_seg, a_loop, mem)
    cp_out(pl.ds((n_seg - group) * seg, group * seg)).start()
    pltpu.make_async_copy(out_ref, out_hbm, out_sem.at[0]).wait()


@functools.partial(jax.jit, static_argnames=("A_seg_len",))
def pallas_gated_mix__memory_aug_recurrent_mem_tr__sliding_local_dilated__prompt_kernel(
    A_x: jax.Array,
    A_mem0: jax.Array,
    A_Wq: jax.Array,
    A_Wk: jax.Array,
    A_Wv: jax.Array,
    A_Wo: jax.Array,
    A_seg_len: int,
    B_x: jax.Array,
    B_wqkv: jax.Array,
    B_wo: jax.Array,
    gate_w: jax.Array,
):
    del B_x
    _, S, D = A_x.shape
    _, H, dh = A_Wq.shape
    M = A_mem0.shape[1]
    seg = int(A_seg_len)
    E = H * dh
    n_pair = H // 2
    t_chunk, t_sub = 256, 128
    group = 9
    assert (S // seg - 1) % group == 0
    n_chunk = S // t_chunk

    def rows_major(w):
        return jnp.transpose(w, (1, 2, 0)).reshape(E, D)

    hbm = pl.BlockSpec(memory_space=pl.ANY)
    vmem = pl.BlockSpec(memory_space=pltpu.VMEM)
    out = pl.pallas_call(
        functools.partial(_kernel, seg=seg, dh=dh, t_chunk=t_chunk, t_sub=t_sub,
                          group=group),
        out_shape=jax.ShapeDtypeStruct((S, D), A_x.dtype),
        in_specs=[hbm, vmem, hbm, hbm, hbm, hbm, hbm, hbm, vmem],
        out_specs=hbm,
        scratch_shapes=[
            pltpu.VMEM((S, D), _BF16),
            pltpu.VMEM((3, E, D), _BF16),
            pltpu.VMEM((n_pair, D, 6 * dh), _BF16),
            pltpu.VMEM((E, D), _BF16),
            pltpu.VMEM((3, D, D), _BF16),
            pltpu.VMEM((D, D), _BF16),
            pltpu.VMEM((4, D // _LANES, D, _LANES), _F32),
            pltpu.VMEM((4, D, D), _BF16),
            pltpu.VMEM((3, D // _LANES, _HALO + S, _LANES), _F32),
            pltpu.VMEM((S, D), _BF16),
            pltpu.VMEM((S, D), _F32),
            pltpu.VMEM((S, _LANES), _F32),
            pltpu.VMEM((S, D), A_x.dtype),
            pltpu.SemaphoreType.DMA((7,)),
            pltpu.SemaphoreType.DMA((n_chunk, 3)),
            pltpu.SemaphoreType.DMA((1,)),
        ],
        compiler_params=pltpu.CompilerParams(vmem_limit_bytes=110 * 1024 * 1024),
    )(A_x.reshape(S, D), A_mem0.reshape(M, D), rows_major(A_Wq), rows_major(A_Wk),
      rows_major(A_Wv), A_Wo.reshape(E, D), B_wqkv, B_wo, gate_w)
    return out.reshape(1, S, D)
```

```python
import functools

import jax
import jax.numpy as jnp
import jax.experimental.pallas as pl
import jax.experimental.pallas.tpu as pltpu

_LANES = 128
_B_HEADS = 32
_B_WIN = 8
_B_DIL = 2
_HALO = 16
_MASKED = -1000000000.0
_F32 = jnp.float32
_BF16 = jnp.bfloat16


_DMA_PLAN = {
    "begin": ((), ("bq", "bk", "x0")),
    (0, 0): (("bq", "bk", "x0"), ("bv", "x1", "bwo")),
    (0, 2): (("bv",), (0,)),
    (1, 0): ((), (1,)),
    (2, 0): (("x1", "bwo", 0), (2, 3)),
    (3, 0): ((1,), (4,)),
    (4, 0): ((2,), (5,)),
    (5, 0): ((3,), (6,)),
    (6, 0): ((4,), (7,)),
    (7, 0): ((5,), ("wo",)),
    (8, 0): ((6, 7), ()),
    "wo": (("wo",), ()),
}
_TRANSPOSE_PLAN = {2: (0,), 3: (1,), 4: (2,), 5: (3,), 6: (4,), 7: (5,), 8: (6, 7)}


def _mm(a, b):
    return jax.lax.dot_general(a, b, (((1,), (0,)), ((), ())),
                               preferred_element_type=_F32)


def _mm_nt(a, b):
    return jax.lax.dot_general(a, b, (((1,), (1,)), ((), ())),
                               preferred_element_type=_F32)


def _iota(shape, dim):
    return jax.lax.broadcasted_iota(jnp.int32, shape, dim)


def _step_order(n):
    ops = []
    lags = (("qk", 0), ("softmax", 1), ("v", 3), ("pv", 9))
    for i in range(n + lags[-1][1]):
        ops += [(op, i - lag) for op, lag in lags if 0 <= i - lag < n]
    return ops


def _kernel(x_hbm, mem0_ref, wq_hbm, wk_hbm, wv_hbm, wo_hbm, bqkv_hbm, bwo_hbm,
            gate_ref, out_hbm,
            x_ref, stage_ref, wt_ref, wo_ref, bqkv_ref, bwo_ref, b32_ref,
            bp_ref, qkv_ref, att_ref, b_ref, g_ref,
            out_ref, in_sem, w_sem, out_sem,
            *, seg, dh, t_chunk, t_sub):
    S, D = x_ref.shape
    M = mem0_ref.shape[0]
    L = M + seg
    n_seg = S // seg
    n_pair, pw = wt_ref.shape[0], 2 * dh
    n_chunk = S // t_chunk
    ppc = n_pair // n_chunk
    n_tile = D // _LANES
    bdh = D // _B_HEADS

    x_head = 2 * t_chunk
    cp = {
        "x0": [pltpu.make_async_copy(x_hbm.at[0:x_head], x_ref.at[0:x_head], in_sem.at[0])],
        "x1": [pltpu.make_async_copy(x_hbm.at[x_head:S], x_ref.at[x_head:S], in_sem.at[1])],
        "bwo": [pltpu.make_async_copy(bwo_hbm, bwo_ref, in_sem.at[2])],
        "wo": [pltpu.make_async_copy(wo_hbm, wo_ref, in_sem.at[3])],
    }
    for m, name in enumerate(("bq", "bk", "bv")):
        cols = slice(m * D, (m + 1) * D)
        cp[name] = [pltpu.make_async_copy(bqkv_hbm.at[:, cols], bqkv_ref.at[m],
                                          in_sem.at[4 + m])]
    for c in range(n_chunk):
        rows = slice(c * ppc * pw, (c + 1) * ppc * pw)
        cp[c] = [pltpu.make_async_copy(src.at[rows], stage_ref.at[m, rows], w_sem.at[c, m])
                 for m, src in enumerate((wq_hbm, wk_hbm, wv_hbm))]

    def dma(point):
        waits, starts = _DMA_PLAN.get(point, ((), ()))
        for name in waits:
            for copy in cp[name]:
                copy.wait()
        for name in starts:
            for copy in cp[name]:
                copy.start()

    dma("begin")

    def reorder_rows(m, tile):
        for j in range(n_tile):
            b32_ref[m, j] = tile(j).astype(_F32)
            for d in range(bdh):
                bp_ref[m, d * _B_HEADS:(d + 1) * _B_HEADS, j * _LANES:(j + 1) * _LANES] = (
                    b32_ref[m, j, pl.ds(d, _B_HEADS, stride=bdh), :].astype(_BF16))

    b_scale = float(bdh) ** -0.5

    def b_project(c, m):
        if c == 0:
            reorder_rows(m, lambda j: bqkv_ref[m, j * _LANES:(j + 1) * _LANES, :].T)
        y = _mm_nt(x_ref[c * t_chunk:(c + 1) * t_chunk, :], bp_ref[m])
        if m == 0:
            y = y * b_scale
        for j in range(n_tile):
            cols = slice(j * _LANES, (j + 1) * _LANES)
            qkv_ref[m, j, _HALO + c * t_chunk:_HALO + (c + 1) * t_chunk, :] = y[:, cols]
            if c == 0 and m > 0:
                qkv_ref[m, j, 0:_HALO, :] = jnp.broadcast_to(y[0:1, cols], (_HALO, _LANES))

    def b_attend(r):
        def rows(m, j, w):
            return qkv_ref[m, j, pl.ds(_HALO + r - w * _B_DIL, t_sub), :]

        q = [rows(0, j, 0) for j in range(n_tile)]
        logits = []
        for w in range(_B_WIN):
            s = functools.reduce(jnp.add, [q[j] * rows(1, j, w) for j in range(n_tile)])
            s = s + pltpu.roll(s, 2 * _B_HEADS, 1)
            s = s + pltpu.roll(s, _B_HEADS, 1)
            if r < w * _B_DIL:
                pos = r + _iota((t_sub, _LANES), 0)
                s = jnp.where(pos >= w * _B_DIL, s, _MASKED)
            logits.append(s)
        mx = functools.reduce(jnp.maximum, logits)
        es = [jnp.exp(s - mx) for s in logits]
        inv = 1.0 / functools.reduce(jnp.add, es)
        for j in range(n_tile):
            acc = functools.reduce(jnp.add, [es[w] * rows(2, j, w) for w in range(_B_WIN)])
            att_ref[r:r + t_sub, j * _LANES:(j + 1) * _LANES] = (acc * inv).astype(_BF16)

    def b_output(c):
        if c == 0:
            reorder_rows(3, lambda j: bwo_ref[:, j * _LANES:(j + 1) * _LANES])
        rows = slice(c * t_chunk, (c + 1) * t_chunk)
        g = jax.nn.sigmoid(jnp.sum(x_ref[rows, :].astype(_F32) * gate_ref[...].astype(_F32).reshape(1, D),
                                   axis=1, keepdims=True))
        g_ref[rows, :] = jnp.broadcast_to(g, (t_chunk, _LANES))
        b_ref[rows, :] = (1.0 - g) * _mm(att_ref[rows, :], bp_ref[3])

    def transpose_w(c, m):
        for p in range(c * ppc, (c + 1) * ppc):
            wt_ref[p, :, m * pw:(m + 1) * pw] = stage_ref[m, p * pw:(p + 1) * pw, :].T

    n_sub = t_chunk // t_sub
    subs = [n_sub * f // 8 for f in (0, 4, 8, 8, 8)]
    for i in range(n_chunk):
        for m in range(4):
            dma((i, m))
            if i >= 1:
                for u in range(subs[m], subs[m + 1]):
                    b_attend((i - 1) * t_chunk + u * t_sub)
            if m < 3:
                for c in _TRANSPOSE_PLAN.get(i, ()):
                    transpose_w(c, m)
            if m < 3:
                b_project(i, m)
            if m == 3 and i >= 2:
                b_output(i - 2)

    dma((n_chunk, 0))
    leftover = [functools.partial(b_attend, r) for r in range(S - t_chunk, S, t_sub)]
    leftover += [functools.partial(transpose_w, c, m)
                 for c in _TRANSPOSE_PLAN[n_chunk] for m in range(3)]
    leftover += [functools.partial(b_output, c) for c in (n_chunk - 2, n_chunk - 1)]

    a_scale = float(dh) ** -0.5

    def seg_rows(s):
        return pl.ds(s * seg if isinstance(s, int) else pl.multiple_of(s * seg, seg), seg)

    def block_diag(t):
        first = _iota((L, pw), 1) < dh
        return jnp.concatenate(
            [jnp.where(first, t, 0.0), jnp.where(first, 0.0, t)], axis=0
        ).astype(_BF16)

    def a_step(s, mem, first_step=False):
        h = jnp.concatenate([mem, x_ref[seg_rows(s), :].astype(_F32)], axis=0)

        row = _iota((L, 2 * L), 0)
        col = _iota((L, 2 * L), 1)
        first = col < L
        key = jnp.where(first, col, col - L)
        visible = (row < M) | (row >= key)

        def softmax(q, kbd):
            sc = jnp.where(visible, _mm_nt(q, kbd) * a_scale, _MASKED)
            m0 = jnp.max(jnp.where(first, sc, -jnp.inf), axis=1, keepdims=True)
            m1 = jnp.max(jnp.where(first, -jnp.inf, sc), axis=1, keepdims=True)
            e = jnp.exp(sc - jnp.where(first, m0, m1))
            s0 = jnp.sum(jnp.where(first, e, 0.0), axis=1, keepdims=True)
            s1 = jnp.sum(jnp.where(first, 0.0, e), axis=1, keepdims=True)
            return e / jnp.where(first, s0, s1)

        qk, v, prob, att = {}, {}, {}, {}
        for op, p in _step_order(n_pair):
            if op == "qk":
                if first_step and p < len(leftover):
                    leftover[p]()
                y = _mm(h, wt_ref[p, :, 0:2 * pw])
                qk[p] = y[:, 0:pw], block_diag(y[:, pw:])
            elif op == "v":
                v[p] = block_diag(_mm(h, wt_ref[p, :, 2 * pw:]))
            elif op == "softmax":
                prob[p] = softmax(*qk[p])
            else:
                att[p] = _mm(prob[p], v[p])
        if first_step:
            dma("wo")
        res = _mm(jnp.concatenate([att[p] for p in range(n_pair)], axis=1), wo_ref[...])
        rows = seg_rows(s)
        g = g_ref[rows, :]
        g = jnp.concatenate([g] * n_tile, axis=1)
        out_ref[rows, :] = (g * res[M:, :] + b_ref[rows, :]).astype(out_ref.dtype)
        return res[0:M, :]

    cp_head, cp_tail = [
        pltpu.make_async_copy(out_ref.at[rows], out_hbm.at[rows], out_sem.at[i])
        for i, rows in enumerate((slice(0, S - seg), slice(S - seg, S)))]

    def a_loop(s, mem):
        @pl.when(s == n_seg - 1)
        def _():
            cp_head.start()
        return a_step(s, mem)

    mem = a_step(0, mem0_ref[...].astype(_F32), first_step=True)
    jax.lax.fori_loop(1, n_seg, a_loop, mem)
    cp_tail.start()
    cp_head.wait()
    cp_tail.wait()


@functools.partial(jax.jit, static_argnames=("A_seg_len",))
def pallas_gated_mix__memory_aug_recurrent_mem_tr__sliding_local_dilated__prompt_kernel(
    A_x: jax.Array,
    A_mem0: jax.Array,
    A_Wq: jax.Array,
    A_Wk: jax.Array,
    A_Wv: jax.Array,
    A_Wo: jax.Array,
    A_seg_len: int,
    B_x: jax.Array,
    B_wqkv: jax.Array,
    B_wo: jax.Array,
    gate_w: jax.Array,
):
    del B_x
    _, S, D = A_x.shape
    _, H, dh = A_Wq.shape
    M = A_mem0.shape[1]
    seg = int(A_seg_len)
    E = H * dh
    n_pair = H // 2
    t_chunk, t_sub = 256, 128
    n_chunk = S // t_chunk

    def rows_major(w):
        return jnp.transpose(w, (1, 2, 0)).reshape(E, D)

    hbm = pl.BlockSpec(memory_space=pl.ANY)
    vmem = pl.BlockSpec(memory_space=pltpu.VMEM)
    out = pl.pallas_call(
        functools.partial(_kernel, seg=seg, dh=dh, t_chunk=t_chunk, t_sub=t_sub),
        out_shape=jax.ShapeDtypeStruct((S, D), A_x.dtype),
        in_specs=[hbm, vmem, hbm, hbm, hbm, hbm, hbm, hbm, vmem],
        out_specs=hbm,
        scratch_shapes=[
            pltpu.VMEM((S, D), _BF16),
            pltpu.VMEM((3, E, D), _BF16),
            pltpu.VMEM((n_pair, D, 6 * dh), _BF16),
            pltpu.VMEM((E, D), _BF16),
            pltpu.VMEM((3, D, D), _BF16),
            pltpu.VMEM((D, D), _BF16),
            pltpu.VMEM((4, D // _LANES, D, _LANES), _F32),
            pltpu.VMEM((4, D, D), _BF16),
            pltpu.VMEM((3, D // _LANES, _HALO + S, _LANES), _F32),
            pltpu.VMEM((S, D), _BF16),
            pltpu.VMEM((S, D), _F32),
            pltpu.VMEM((S, _LANES), _F32),
            pltpu.VMEM((S, D), A_x.dtype),
            pltpu.SemaphoreType.DMA((7,)),
            pltpu.SemaphoreType.DMA((n_chunk, 3)),
            pltpu.SemaphoreType.DMA((2,)),
        ],
        compiler_params=pltpu.CompilerParams(vmem_limit_bytes=110 * 1024 * 1024),
    )(A_x.reshape(S, D), A_mem0.reshape(M, D), rows_major(A_Wq), rows_major(A_Wk),
      rows_major(A_Wv), A_Wo.reshape(E, D), B_wqkv, B_wo, gate_w)
    return out.reshape(1, S, D)
```

```python
import functools

import jax
import jax.numpy as jnp
import jax.experimental.pallas as pl
import jax.experimental.pallas.tpu as pltpu

_LANES = 128
_B_HEADS = 32
_B_WIN = 8
_B_DIL = 2
_HALO = 16
_MASKED = -1000000000.0
_F32 = jnp.float32
_BF16 = jnp.bfloat16


_DMA_PLAN = {
    "begin": ((), ("bq", "bk", "x0")),
    (0, 0): (("bq", "bk", "x0"), ("bv", "x1", "bwo")),
    (0, 2): (("bv",), (0,)),
    (1, 0): ((), (1,)),
    (2, 0): (("x1", "bwo", 0), (2, 3)),
    (3, 0): ((1,), (4,)),
    (4, 0): ((2,), (5,)),
    (5, 0): ((3,), (6,)),
    (6, 0): ((4,), (7,)),
    (7, 0): ((5,), ("wo",)),
    (8, 0): ((6, 7), ()),
    "wo": (("wo",), ()),
}
_TRANSPOSE_PLAN = {2: (0,), 3: (1,), 4: (2,), 5: (3,), 6: (4,), 7: (5,), 8: (6, 7)}


def _mm(a, b):
    return jax.lax.dot_general(a, b, (((1,), (0,)), ((), ())),
                               preferred_element_type=_F32)


def _mm_nt(a, b):
    return jax.lax.dot_general(a, b, (((1,), (1,)), ((), ())),
                               preferred_element_type=_F32)


def _iota(shape, dim):
    return jax.lax.broadcasted_iota(jnp.int32, shape, dim)


def _step_order(n):
    ops = []
    lags = (("qk", 0), ("softmax", 1), ("v", 3), ("pv", 9))
    for i in range(n + lags[-1][1]):
        ops += [(op, i - lag) for op, lag in lags if 0 <= i - lag < n]
    return ops


def _kernel(x_hbm, mem0_ref, wq_hbm, wk_hbm, wv_hbm, wo_hbm, bqkv_hbm, bwo_hbm,
            gate_ref, out_hbm,
            x_ref, stage_ref, wt_ref, wo_ref, bqkv_ref, bwo_ref, b32_ref,
            bp_ref, qkv_ref, att_ref, b_ref, g_ref,
            out_ref, in_sem, w_sem, out_sem,
            *, seg, dh, t_chunk, t_sub):
    S, D = x_ref.shape
    M = mem0_ref.shape[0]
    L = M + seg
    n_seg = S // seg
    n_pair, pw = wt_ref.shape[0], 2 * dh
    n_chunk = S // t_chunk
    ppc = n_pair // n_chunk
    n_tile = D // _LANES
    bdh = D // _B_HEADS

    x_head = 2 * t_chunk
    cp = {
        "x0": [pltpu.make_async_copy(x_hbm.at[0:x_head], x_ref.at[0:x_head], in_sem.at[0])],
        "x1": [pltpu.make_async_copy(x_hbm.at[x_head:S], x_ref.at[x_head:S], in_sem.at[1])],
        "bwo": [pltpu.make_async_copy(bwo_hbm, bwo_ref, in_sem.at[2])],
        "wo": [pltpu.make_async_copy(wo_hbm, wo_ref, in_sem.at[3])],
    }
    for m, name in enumerate(("bq", "bk", "bv")):
        cols = slice(m * D, (m + 1) * D)
        cp[name] = [pltpu.make_async_copy(bqkv_hbm.at[:, cols], bqkv_ref.at[m],
                                          in_sem.at[4 + m])]
    for c in range(n_chunk):
        rows = slice(c * ppc * pw, (c + 1) * ppc * pw)
        cp[c] = [pltpu.make_async_copy(src.at[rows], stage_ref.at[m, rows], w_sem.at[c, m])
                 for m, src in enumerate((wq_hbm, wk_hbm, wv_hbm))]

    def dma(point):
        waits, starts = _DMA_PLAN.get(point, ((), ()))
        for name in waits:
            for copy in cp[name]:
                copy.wait()
        for name in starts:
            for copy in cp[name]:
                copy.start()

    dma("begin")

    def reorder_rows(m, tile):
        for j in range(n_tile):
            b32_ref[m, j, 0:D, :] = tile(j).astype(_F32)
            for d in range(bdh):
                bp_ref[m, d * _B_HEADS:(d + 1) * _B_HEADS, j * _LANES:(j + 1) * _LANES] = (
                    b32_ref[m, j, pl.ds(d, _B_HEADS, stride=bdh), :].astype(_BF16))

    b_scale = float(bdh) ** -0.5

    def b_project(c, m):
        if c == 0:
            reorder_rows(m, lambda j: bqkv_ref[m, j * _LANES:(j + 1) * _LANES, :].T)
        y = _mm_nt(x_ref[c * t_chunk:(c + 1) * t_chunk, :], bp_ref[m])
        if m == 0:
            y = y * b_scale
        for j in range(n_tile):
            cols = slice(j * _LANES, (j + 1) * _LANES)
            qkv_ref[m, j, _HALO + c * t_chunk:_HALO + (c + 1) * t_chunk, :] = y[:, cols]
            if c == 0 and m > 0:
                qkv_ref[m, j, 0:_HALO, :] = jnp.broadcast_to(y[0:1, cols], (_HALO, _LANES))

    def b_attend(r):
        def rows(m, j, w):
            return qkv_ref[m, j, pl.ds(_HALO + r - w * _B_DIL, t_sub), :]

        q = [rows(0, j, 0) for j in range(n_tile)]
        logits = []
        for w in range(_B_WIN):
            s = functools.reduce(jnp.add, [q[j] * rows(1, j, w) for j in range(n_tile)])
            s = s + pltpu.roll(s, 2 * _B_HEADS, 1)
            s = s + pltpu.roll(s, _B_HEADS, 1)
            if r < w * _B_DIL:
                pos = r + _iota((t_sub, _LANES), 0)
                s = jnp.where(pos >= w * _B_DIL, s, _MASKED)
            logits.append(s)
        mx = functools.reduce(jnp.maximum, logits)
        es = [jnp.exp(s - mx) for s in logits]
        inv = 1.0 / functools.reduce(jnp.add, es)
        for j in range(n_tile):
            acc = functools.reduce(jnp.add, [es[w] * rows(2, j, w) for w in range(_B_WIN)])
            att_ref[r:r + t_sub, j * _LANES:(j + 1) * _LANES] = (acc * inv).astype(_BF16)

    def b_output(c):
        if c == 0:
            reorder_rows(3, lambda j: bwo_ref[:, j * _LANES:(j + 1) * _LANES])
        rows = slice(c * t_chunk, (c + 1) * t_chunk)
        gate = gate_ref[...].astype(_F32).reshape(1, D)
        g = jax.nn.sigmoid(jnp.sum(x_ref[rows, :].astype(_F32) * gate, axis=1, keepdims=True))
        g_ref[rows, :] = jnp.broadcast_to(g, (t_chunk, _LANES))
        b_ref[rows, :] = (1.0 - g) * _mm(att_ref[rows, :], bp_ref[3])

    def transpose_w(c, m):
        for p in range(c * ppc, (c + 1) * ppc):
            wt_ref[p, :, m * pw:(m + 1) * pw] = stage_ref[m, p * pw:(p + 1) * pw, :].T

    for i in range(n_chunk):
        for m in range(4):
            dma((i, m))
            if i >= 1 and m * t_sub < t_chunk:
                b_attend((i - 1) * t_chunk + m * t_sub)
            if m >= 2:
                for c in _TRANSPOSE_PLAN.get(i, ()):
                    for mm in ((0, 1), (2,))[m - 2]:
                        transpose_w(c, mm)
            if m < 3:
                b_project(i, m)
            if m == 3 and i >= 2:
                b_output(i - 2)

    dma((n_chunk, 0))
    leftover = [functools.partial(b_attend, r) for r in range(S - t_chunk, S, t_sub)]
    leftover += [functools.partial(transpose_w, c, m)
                 for c in _TRANSPOSE_PLAN[n_chunk] for m in range(3)]
    leftover += [functools.partial(b_output, c) for c in (n_chunk - 2, n_chunk - 1)]

    a_scale = float(dh) ** -0.5

    def seg_rows(s):
        return pl.ds(s * seg if isinstance(s, int) else pl.multiple_of(s * seg, seg), seg)

    def block_diag(t):
        first = _iota((L, pw), 1) < dh
        return jnp.concatenate(
            [jnp.where(first, t, 0.0), jnp.where(first, 0.0, t)], axis=0
        ).astype(_BF16)

    def a_step(s, mem, first_step=False):
        h = jnp.concatenate([mem, x_ref[seg_rows(s), :].astype(_F32)], axis=0)

        row = _iota((L, 2 * L), 0)
        col = _iota((L, 2 * L), 1)
        first = col < L
        key = jnp.where(first, col, col - L)
        visible = (row < M) | (row >= key)

        def softmax(q, kbd):
            sc = jnp.where(visible, _mm_nt(q, kbd) * a_scale, _MASKED)
            m0 = jnp.max(jnp.where(first, sc, -jnp.inf), axis=1, keepdims=True)
            m1 = jnp.max(jnp.where(first, -jnp.inf, sc), axis=1, keepdims=True)
            e = jnp.exp(sc - jnp.where(first, m0, m1))
            s0 = jnp.sum(jnp.where(first, e, 0.0), axis=1, keepdims=True)
            s1 = jnp.sum(jnp.where(first, 0.0, e), axis=1, keepdims=True)
            return e / jnp.where(first, s0, s1)

        qk, v, prob, att = {}, {}, {}, {}
        for op, p in _step_order(n_pair):
            if op == "qk":
                if first_step and p < len(leftover):
                    leftover[p]()
                y = _mm(h, wt_ref[p, :, 0:2 * pw])
                qk[p] = y[:, 0:pw], block_diag(y[:, pw:])
            elif op == "v":
                v[p] = block_diag(_mm(h, wt_ref[p, :, 2 * pw:]))
            elif op == "softmax":
                prob[p] = softmax(*qk[p])
            else:
                att[p] = _mm(prob[p], v[p])
        if first_step:
            dma("wo")
        res = _mm(jnp.concatenate([att[p] for p in range(n_pair)], axis=1), wo_ref[...])
        rows = seg_rows(s)
        g = g_ref[rows, :]
        g = jnp.concatenate([g] * n_tile, axis=1)
        out_ref[rows, :] = (g * res[M:, :] + b_ref[rows, :]).astype(out_ref.dtype)
        return res[0:M, :]

    cp_head, cp_tail = [
        pltpu.make_async_copy(out_ref.at[rows], out_hbm.at[rows], out_sem.at[i])
        for i, rows in enumerate((slice(0, S - seg), slice(S - seg, S)))]

    def a_loop(s, mem):
        @pl.when(s == n_seg - 1)
        def _():
            cp_head.start()
        return a_step(s, mem)

    mem = a_step(0, mem0_ref[...].astype(_F32), first_step=True)
    jax.lax.fori_loop(1, n_seg, a_loop, mem)
    cp_tail.start()
    cp_head.wait()
    cp_tail.wait()


@functools.partial(jax.jit, static_argnames=("A_seg_len",))
def pallas_gated_mix__memory_aug_recurrent_mem_tr__sliding_local_dilated__prompt_kernel(
    A_x: jax.Array,
    A_mem0: jax.Array,
    A_Wq: jax.Array,
    A_Wk: jax.Array,
    A_Wv: jax.Array,
    A_Wo: jax.Array,
    A_seg_len: int,
    B_x: jax.Array,
    B_wqkv: jax.Array,
    B_wo: jax.Array,
    gate_w: jax.Array,
):
    del B_x
    _, S, D = A_x.shape
    _, H, dh = A_Wq.shape
    M = A_mem0.shape[1]
    seg = int(A_seg_len)
    E = H * dh
    n_pair = H // 2
    t_chunk, t_sub = 256, 128
    n_chunk = S // t_chunk
    assert A_x.shape[0] == 1 and S == 8 * t_chunk and n_pair == 2 * n_chunk
    assert S % seg == 0 and D % _LANES == 0 and (2 * dh) % _LANES == 0

    def rows_major(w):
        return jnp.transpose(w, (1, 2, 0)).reshape(E, D)

    hbm = pl.BlockSpec(memory_space=pl.ANY)
    vmem = pl.BlockSpec(memory_space=pltpu.VMEM)
    out = pl.pallas_call(
        functools.partial(_kernel, seg=seg, dh=dh, t_chunk=t_chunk, t_sub=t_sub),
        out_shape=jax.ShapeDtypeStruct((S, D), A_x.dtype),
        in_specs=[hbm, vmem, hbm, hbm, hbm, hbm, hbm, hbm, vmem],
        out_specs=hbm,
        scratch_shapes=[
            pltpu.VMEM((S, D), _BF16),
            pltpu.VMEM((3, E, D), _BF16),
            pltpu.VMEM((n_pair, D, 6 * dh), _BF16),
            pltpu.VMEM((E, D), _BF16),
            pltpu.VMEM((3, D, D), _BF16),
            pltpu.VMEM((D, D), _BF16),
            pltpu.VMEM((4, D // _LANES, D + 24, _LANES), _F32),
            pltpu.VMEM((4, D, D), _BF16),
            pltpu.VMEM((3, D // _LANES, _HALO + S, _LANES), _F32),
            pltpu.VMEM((S, D), _BF16),
            pltpu.VMEM((S, D), _F32),
            pltpu.VMEM((S, _LANES), _F32),
            pltpu.VMEM((S, D), A_x.dtype),
            pltpu.SemaphoreType.DMA((7,)),
            pltpu.SemaphoreType.DMA((n_chunk, 3)),
            pltpu.SemaphoreType.DMA((2,)),
        ],
        compiler_params=pltpu.CompilerParams(vmem_limit_bytes=110 * 1024 * 1024),
    )(A_x.reshape(S, D), A_mem0.reshape(M, D), rows_major(A_Wq), rows_major(A_Wk),
      rows_major(A_Wv), A_Wo.reshape(E, D), B_wqkv, B_wo, gate_w)
    return out.reshape(1, S, D)
```
